```python
import jax
import jax.numpy as jnp

def _softmax(x, axis=-1):
    return jax.nn.softmax(x, axis=axis)

def _gelu(x):
    return jax.nn.gelu(x, approximate=True)

def _silu(x):
    return jax.nn.silu(x)

def _sigmoid(x):
    return jax.nn.sigmoid(x)

def _layernorm(x, axis=-1, eps=1e-05):
    m = jnp.mean(x, axis=axis, keepdims=True)
    v = jnp.var(x, axis=axis, keepdims=True)
    return (x - m) / jnp.sqrt(v + eps)

def _scatter_add(tgt, idx, src, axis=0):
    return tgt.at[idx].add(src)

def _segment_sum(src, seg, n):
    return jax.ops.segment_sum(src, seg, n)

class _Rng:

    def __init__(self, key):
        self._k = key

    def _next(self):
        self._k, sub = jax.random.split(self._k)
        return sub

    def normal(self, shape):
        return jax.random.normal(self._next(), shape, dtype=jnp.bfloat16)

    def randint(self, lo, hi, shape):
        return jax.random.randint(self._next(), shape, lo, hi, dtype=jnp.int32)

    def uniform(self, shape, lo=0.0, hi=1.0):
        return jax.random.uniform(self._next(), shape, jnp.bfloat16, lo, hi)

    def permutation(self, n):
        return jax.random.permutation(self._next(), n)
kernel_name = 'sequential_preLN__memory_aug_recurrent_mem_tr__mixer_s_mlp__prompt'

def setup_inputs():
    _rng = _Rng(jax.random.key(int.from_bytes(__import__("os").urandom(4), "little")))
    _w = lambda a: (lambda t: t.astype(jnp.bfloat16) if jnp.issubdtype(t.dtype, jnp.floating) else t)(jnp.asarray(a))

    def _A_setup():
        B, S, Dm = (1, 2048, 1024)
        H, Dh = (32, 128)
        M, seg = (8, 32)
        seg = min(seg, S)
        S = S // seg * seg
        return {'x': _w((lambda *s: _rng.normal(s) * 0.05)(B, S, Dm)), 'mem0': _w((lambda *s: _rng.normal(s) * 0.05)(B, M, Dm)), 'Wq': _w((lambda *s: _rng.normal(s) * 0.05)(Dm, H, Dh) * Dm ** (-0.5)), 'Wk': _w((lambda *s: _rng.normal(s) * 0.05)(Dm, H, Dh) * Dm ** (-0.5)), 'Wv': _w((lambda *s: _rng.normal(s) * 0.05)(Dm, H, Dh) * Dm ** (-0.5)), 'Wo': _w((lambda *s: _rng.normal(s) * 0.05)(H, Dh, Dm) * (H * Dh) ** (-0.5)), 'seg_len': seg}
    _A_in = _A_setup()

    def _B_setup():
        B, S, D, F = (1, 2048, 1024, 3584)
        return {'x': _w((lambda *s: _rng.normal(s) * 0.05)(B, S, D)), 'w1': _w((lambda *s: _rng.normal(s) * 0.05)(D, D) * D ** (-0.5)), 'w2': _w((lambda *s: _rng.normal(s) * 0.05)(D, D) * D ** (-0.5)), 'w3': _w((lambda *s: _rng.normal(s) * 0.05)(D, F) * D ** (-0.5)), 'w4': _w((lambda *s: _rng.normal(s) * 0.05)(F, D) * F ** (-0.5))}
    _B_in = _B_setup()
    return {'A_x': _A_in['x'], 'A_mem0': _A_in['mem0'], 'A_Wq': _A_in['Wq'], 'A_Wk': _A_in['Wk'], 'A_Wv': _A_in['Wv'], 'A_Wo': _A_in['Wo'], 'A_seg_len': _A_in['seg_len'], 'B_x': _B_in['x'], 'B_w1': _B_in['w1'], 'B_w2': _B_in['w2'], 'B_w3': _B_in['w3'], 'B_w4': _B_in['w4']}

def reference(A_x, A_mem0, A_Wq, A_Wk, A_Wv, A_Wo, A_seg_len, B_x, B_w1, B_w2, B_w3, B_w4):

    def _A_ref(x, mem0, Wq, Wk, Wv, Wo, seg_len):
        B, S, Dm = x.shape
        H, Dh = (Wq.shape[1], Wq.shape[2])
        M = mem0.shape[1]
        scale = Dh ** (-0.5)
        n_seg = S // seg_len
        L = M + seg_len
        idx = jnp.arange(L)
        mask = (idx[:, None] < M) | (idx[:, None] >= idx[None, :])
        mem = mem0
        outs = []
        for s in range(n_seg):
            xs = x[:, s * seg_len:(s + 1) * seg_len, :].copy()
            h = jnp.concatenate([mem, xs], axis=1)
            q = jnp.einsum('btd,dhe->bhte', h, Wq)
            k = jnp.einsum('btd,dhe->bhte', h, Wk)
            v = jnp.einsum('btd,dhe->bhte', h, Wv)
            scores = jnp.einsum('bhqe,bhke->bhqk', q, k) * scale
            scores = jnp.where(mask[None, None], scores, -1000000000.0)
            p = _softmax(scores, axis=-1)
            o = jnp.einsum('bhqk,bhke->bhqe', p, v)
            o = jnp.einsum('bhte,hed->btd', o, Wo)
            mem = o[:, :M, :].copy()
            outs.append(o[:, M:, :])
        return jnp.concatenate(outs, axis=1)

    def _B_ref(x, w1, w2, w3, w4):
        B, S, D = x.shape
        h = _gelu(_layernorm(x, axis=-1) @ w1)
        c = D // 4
        g0 = jnp.pad(h[:, :, 0 * c:1 * c], ((0, 0), (1, 0), (0, 0)))[:, :S, :]
        g1 = jnp.pad(h[:, :, 1 * c:2 * c], ((0, 0), (0, 1), (0, 0)))[:, 1:, :]
        g2 = jnp.pad(h[:, :, 2 * c:3 * c], ((0, 0), (2, 0), (0, 0)))[:, :S, :]
        g3 = jnp.pad(h[:, :, 3 * c:], ((0, 0), (0, 2), (0, 0)))[:, 2:, :]
        hs = jnp.concatenate([g0, g1, g2, g3], axis=-1) @ w2
        x1 = x + hs
        h2 = _gelu(_layernorm(x1, axis=-1) @ w3) @ w4
        return x1 + h2
    x = A_x
    h = x + _A_ref(_layernorm(x, axis=-1), A_mem0, A_Wq, A_Wk, A_Wv, A_Wo, A_seg_len)
    h2 = h + _B_ref(_layernorm(h, axis=-1), B_w1, B_w2, B_w3, B_w4)
    return h2
```

```python
import functools
import jax
import jax.numpy as jnp
from jax.experimental import pallas as pl
from jax.experimental.pallas import tpu as pltpu

F32 = jnp.float32
BF16 = jnp.bfloat16
U32 = jnp.uint32
EPS = 1e-5


def _ln(x):
    m = jnp.mean(x, axis=-1, keepdims=True)
    xc = x - m
    v = jnp.mean(xc * xc, axis=-1, keepdims=True)
    return xc * jax.lax.rsqrt(v + EPS)


def _gelu(x):
    c = 0.7978845608028654
    return 0.5 * x * (1.0 + jnp.tanh(c * (x + 0.044715 * (x * x * x))))


def _dot(a, b):
    return jnp.dot(a, b, preferred_element_type=F32)


def _b(x):
    return pltpu.bitcast(x, BF16)


def _u(x):
    return pltpu.bitcast(x, U32)


def default_sched(H):
    s = {}
    def add(p, it, *names):
        s.setdefault((p, it), []).extend(names)
    add(1, 0, ('ln1',))
    for n in range(8):
        add(1, 2 + n, ('w1', n))
    add(1, 11, ('mix',))
    for n in range(8):
        add(1, 13 + n, ('w2', n))
    add(1, 22, ('ln2',))
    w3 = list(range(28))
    pos = [(1, i) for i in range(25, 32)] + [(1, 32)] * 3 + [(1, 33)] * 2 + [(1, 34)] * 2 + [(2, i) for i in range(0, 14)]
    assert len(pos) == 28
    for n, (p, it) in zip(w3, pos):
        add(p, it, ('w3', n))
    pos4 = [(2, 16), (2, 19), (2, 22), (2, 25), (2, 28), (2, 32), (2, 33), (2, 34)]
    for n, (p, it) in enumerate(pos4):
        add(p, it, ('w4', n))
    return s


def make_kernel(S, D, H, E, M, SEG, FF, G, do_b=True, nrun=None):
    assert SEG == 32 and M == 8
    NSEG = S // SEG
    NSUP = NSEG // 2
    RB = 2 * SEG
    LP = SEG + 16
    scale = float(E) ** -0.5
    DC = 128
    NT = D // 128
    NF = FF // 128
    PADB = 0
    PH = 8
    C4 = D // 4
    sched = default_sched(H)

    def kernel(x_hbm, mem0_hbm, wq_hbm, wk_hbm, wv_hbm, wo_hbm, w1_hbm, w2_hbm, w3_hbm, w4_hbm,
               out_hbm,
               x_v, xn_v, h_v, h1_v, wq_v, wk_v, wv_v, wo_v, w1_v, w2_v, w3_v, w4_v,
               stage, stage2, mem_v, lhs1_v, lhs2_v, qs_v, os_v, o1_v, o2_v, acc1_v, acc2_v,
               bl_v, x1_v, t_v, out_v, sems):
        cp_x = pltpu.make_async_copy(x_hbm.at[0], x_v, sems.at[0]); cp_x.start()
        cp_m = pltpu.make_async_copy(mem0_hbm.at[0], mem_v, sems.at[1]); cp_m.start()
        srcs = [wq_hbm, wk_hbm, wv_hbm]
        NCH = D // DC
        chunks = [(w, c) for w in range(3) for c in range(NCH)]
        NST = stage.shape[0]
        def stage_cp(i):
            w, c = chunks[i]
            return pltpu.make_async_copy(srcs[w].at[pl.ds(c * DC, DC)], stage.at[i % NST], sems.at[8 + i % NST])
        NST2, R2 = stage2.shape[0], stage2.shape[1]
        NCH2 = H * E // R2
        def stage2_cp(i):
            return pltpu.make_async_copy(wo_hbm.at[pl.ds(i * R2, R2)], stage2.at[i % NST2], sems.at[8 + NST + i % NST2])
        for i in range(NST):
            stage_cp(i).start()
        cps = [pltpu.make_async_copy(s, d, sems.at[3 + i]) for i, (s, d) in enumerate(
            [(w1_hbm, w1_v), (w2_hbm, w2_v), (w3_hbm, w3_v), (w4_hbm, w4_v)])]
        h1_v[pl.ds(0, PH), :] = jnp.zeros((PH, D), F32)
        h1_v[pl.ds(PH + S, 8), :] = jnp.zeros((8, D), F32)
        cp_x.wait()
        def ln_body(i, c):
            r0 = pl.multiple_of(i * 32, 32)
            xn_v[pl.ds(r0, 32), :] = _ln(x_v[pl.ds(r0, 32), :].astype(F32)).astype(BF16)
            return c
        jax.lax.fori_loop(0, S // 32, ln_body, 0)
        dsts = [wq_v, wk_v, wv_v]
        for i in range(len(chunks)):
            stage_cp(i).wait()
            w, c = chunks[i]
            def rl(t, carry, i=i, w=w, c=c):
                t0 = pl.multiple_of(t * 16, 16)
                v = stage[i % NST, pl.ds(t0, 16)]
                dsts[w][:, pl.ds(pl.multiple_of(c * (DC // 2) + t * 8, 8), 8), :] = _u(jnp.swapaxes(v, 0, 1))
                return carry
            jax.lax.fori_loop(0, DC // 16, rl, 0)
            if i + NST < len(chunks):
                stage_cp(i + NST).start()
            else:
                j = i + NST - len(chunks)
                if j < NST2:
                    stage2_cp(j).start()
        for j in range(NST, NST2):
            stage2_cp(j).start()
        for j in range(NCH2):
            stage2_cp(j).wait()
            def cv(t, carry, j=j):
                t0 = pl.multiple_of(t * 16, 16)
                wo_v[pl.ds(pl.multiple_of(j * (R2 // 2) + t * 8, 8), 8), :] = _u(stage2[j % NST2, pl.ds(t0, 16), :])
                return carry
            jax.lax.fori_loop(0, R2 // 16, cv, 0)
            if j + NST2 < NCH2:
                stage2_cp(j + NST2).start()
        for cp in cps:
            cp.start()
        cp_m.wait()

        row = jax.lax.broadcasted_iota(jnp.int32, (LP, LP), 0)
        col = jax.lax.broadcasted_iota(jnp.int32, (LP, LP), 1)
        allowed = (col < SEG + M) & ((row >= SEG) | (col >= SEG) | (col <= row))

        def set_lhs1(k, mem):
            r0 = pl.multiple_of(k * RB, RB)
            lhs1_v[pl.ds(0, 16), :] = _u(xn_v[pl.ds(r0, SEG), :])
            tb = xn_v[pl.ds(r0 + SEG, 8), :].astype(F32)
            lhs1_v[pl.ds(16, 8), :] = _u(jnp.concatenate([mem, tb], axis=0).astype(BF16))

        def set_lhs2(k, mem):
            r0 = pl.multiple_of(k * RB, RB)
            t = xn_v[pl.ds(r0 + SEG + 8, 24), :].astype(F32)
            lhs2_v[...] = _u(jnp.concatenate([t, mem], axis=0).astype(BF16))

        def b_ops(j1, j2):
            r1 = pl.multiple_of(PADB + j1 * RB, RB)
            r2 = pl.multiple_of(PADB + j2 * RB, RB)

            def ln1():
                for c in range(RB // 16):
                    hb = h_v[pl.ds(r1 + 16 * c, 16), :]
                    bl_v[0, pl.ds(8 * c, 8), :] = _u(_ln(_ln(hb)).astype(BF16))

            def w1(n):
                y = _dot(_b(bl_v[0]), w1_v[:, n * 128:(n + 1) * 128])
                h1_v[pl.ds(r1 + PH, RB), n * 128:(n + 1) * 128] = _gelu(y)

            def mix():
                offs = [-1, 1, -2, 2]
                for g in range(4):
                    win = h1_v[pl.ds(r2, RB + 16), g * C4:(g + 1) * C4]
                    sh = win[8 + offs[g]:8 + offs[g] + RB]
                    bl_v[1, :, g * C4:(g + 1) * C4] = _u(sh.astype(BF16))

            def w2(n):
                y = _dot(_b(bl_v[1]), w2_v[:, n * 128:(n + 1) * 128])
                x1_v[:, n * 128:(n + 1) * 128] = y

            def ln2():
                for c in range(RB // 16):
                    hb = h_v[pl.ds(r2 + 16 * c, 16), :]
                    x1 = _ln(hb) + x1_v[pl.ds(16 * c, 16), :]
                    x1_v[pl.ds(16 * c, 16), :] = hb + x1
                    bl_v[2, pl.ds(8 * c, 8), :] = _u(_ln(x1).astype(BF16))

            def w3(n):
                y = _dot(_b(bl_v[2]), w3_v[:, n * 128:(n + 1) * 128])
                t_v[:, n * 128:(n + 1) * 128] = _u(_gelu(y).astype(BF16))

            def w4(n):
                y = _dot(_b(t_v[...]), w4_v[:, n * 128:(n + 1) * 128])
                out_v[pl.ds(r2, RB), n * 128:(n + 1) * 128] = (x1_v[:, n * 128:(n + 1) * 128] + y).astype(BF16)

            return dict(ln1=ln1, w1=w1, mix=mix, w2=w2, ln2=ln2, w3=w3, w4=w4)

        def phase(p, k, bops):
            lhs_v = lhs1_v if p == 1 else lhs2_v
            o_v = o1_v if p == 1 else o2_v
            acc_v = acc1_v if p == 1 else acc2_v
            qb, kb, vb, pb, rinv = {}, {}, {}, {}, {}

            def proj(w_ref, h, idx, mul=None):
                y = _dot(_b(lhs_v[...]), _b(w_ref[h]))
                if mul is not None:
                    y = y * mul
                cs = slice(h * E, (h + 1) * E)
                if p == 1:
                    qs_v[idx, :, cs] = y[40:48]
                    return y.astype(BF16)
                full = jnp.concatenate([qs_v[idx, :, cs], y, jnp.zeros((8, E), F32)], axis=0)
                return full.astype(BF16)

            def qk(h):
                sc = jax.lax.dot_general(qb.pop(h), kb.pop(h), (((1,), (1,)), ((), ())),
                                         preferred_element_type=F32)
                sc = jnp.where(allowed, sc, -1e30)
                mx = jnp.max(sc, axis=-1, keepdims=True)
                pe = jnp.exp(sc - mx)
                rinv[h] = pl.reciprocal(jnp.sum(pe, axis=-1, keepdims=True), approx=False)
                pb[h] = pe.astype(BF16)

            def pv(h):
                o = _dot(pb.pop(h), vb.pop(h)) * rinv.pop(h)
                cs = slice(h * E, (h + 1) * E)
                if p == 1:
                    o_v[:, cs] = _u(jnp.concatenate([o[0:24], o[32:40]], axis=0).astype(BF16))
                    os_v[:, cs] = o[24:32]
                else:
                    o_v[:, cs] = _u(jnp.concatenate([o[0:40], os_v[:, cs]], axis=0).astype(BF16))

            def wo_group(g):
                k0 = g * G * E
                og = _b(o_v[:, k0:k0 + G * E])
                for n in range(NT):
                    y = _dot(og, _b(wo_v[k0 // 2:(k0 + G * E) // 2, n * 128:(n + 1) * 128]))
                    if g == 0:
                        acc_v[:, n * 128:(n + 1) * 128] = y
                    else:
                        acc_v[:, n * 128:(n + 1) * 128] += y

            def fin():
                r0 = pl.multiple_of(k * RB, RB)
                if p == 1:
                    h_v[pl.ds(PADB + r0, 24), :] = x_v[pl.ds(r0, 32), :].astype(F32)[0:24] + acc_v[pl.ds(0, 24), :]
                    set_lhs2(k, acc_v[pl.ds(24, 8), :])
                else:
                    xa = x_v[pl.ds(r0 + 16, 16), :].astype(F32)[8:16]
                    h_v[pl.ds(PADB + r0 + 24, 8), :] = xa + acc_v[pl.ds(40, 8), :]
                    h_v[pl.ds(PADB + r0 + 32, 32), :] = x_v[pl.ds(r0 + 32, 32), :].astype(F32) + acc_v[pl.ds(0, 32), :]
                    kn = jnp.minimum(k + 1, NSUP - 1)
                    set_lhs1(kn, acc_v[pl.ds(32, 8), :])

            def emit_b(it):
                if bops is None:
                    return
                for op in sched.get((p, it), []):
                    bops[op[0]](*op[1:])

            for it in range(H + 3):
                if it < H:
                    qb[it] = proj(wq_v, it, 0, scale)
                if 0 <= it - 1 < H:
                    qk(it - 1)
                if it < H:
                    kb[it] = proj(wk_v, it, 1)
                if 0 <= it - 2 < H:
                    pv(it - 2)
                if it < H:
                    vb[it] = proj(wv_v, it, 2)
                h3 = it - 3
                if 0 <= h3 < H and h3 % G == G - 1:
                    wo_group(h3 // G)
                if it == H + 2:
                    fin()
                emit_b(it)

        def out_cp(j):
            r = pl.multiple_of(j * RB, RB)
            return pltpu.make_async_copy(out_v.at[pl.ds(r, RB)], out_hbm.at[0, pl.ds(r, RB)], sems.at[7])

        def run_ops(bops, names):
            for op in names:
                if isinstance(op, str):
                    bops[op]()
                else:
                    bops[op[0]](*op[1:])

        def a_body(k, c):
            phase(1, k, None)
            phase(2, k, None)
            return c

        def sup_body(k, c):
            bops = b_ops(k - 1, k - 2)
            phase(1, k, bops)
            phase(2, k, bops)
            out_cp(k - 2).start()
            return c

        set_lhs1(0, mem_v[...].astype(F32))
        jax.lax.fori_loop(0, 2, a_body, 0)
        st1 = ['ln1'] + [('w1', n) for n in range(NT)]
        st2 = ['mix'] + [('w2', n) for n in range(NT)] + ['ln2'] \
            + [('w3', n) for n in range(NF)] + [('w4', n) for n in range(NT)]
        cps[0].wait()
        run_ops(b_ops(0, 0), st1)
        for cp in cps[1:]:
            cp.wait()
        NRUN = NSUP if nrun is None else nrun
        jax.lax.fori_loop(2, NRUN, sup_body, 0)

        run_ops(b_ops(NSUP - 1, NSUP - 2), st1 + st2)
        out_cp(NSUP - 2).start()
        run_ops(b_ops(NSUP - 1, NSUP - 1), st2)
        out_cp(NSUP - 1).start()
        for j in range(NRUN - 2):
            out_cp(j).wait()
        out_cp(NSUP - 2).wait()
        out_cp(NSUP - 1).wait()

    return kernel


@functools.partial(jax.jit, static_argnames=("A_seg_len",))
def pallas_sequential_preLN__memory_aug_recurrent_mem_tr__mixer_s_mlp__prompt_kernel(
    A_x, A_mem0, A_Wq, A_Wk, A_Wv, A_Wo, A_seg_len, B_x, B_w1, B_w2, B_w3, B_w4):
    x, mem0, wq, wk, wv, wo = A_x, A_mem0, A_Wq, A_Wk, A_Wv, A_Wo
    w1, w2, w3, w4 = B_w1, B_w2, B_w3, B_w4
    seg, G, do_b, nrun = int(A_seg_len), 4, True, None
    B, S, D = x.shape
    _, H, E = wq.shape
    M = mem0.shape[1]
    FF = w3.shape[1]
    wo2 = wo.reshape(H * E, D)
    NST = 4
    NST2 = 4
    RB = 2 * seg
    PADB = 0
    kernel = make_kernel(S, D, H, E, M, seg, FF, G, do_b, nrun)
    anyspec = pl.BlockSpec(memory_space=pl.ANY)
    return pl.pallas_call(
        kernel,
        out_shape=jax.ShapeDtypeStruct((B, S, D), BF16),
        in_specs=[anyspec] * 10,
        out_specs=anyspec,
        scratch_shapes=[
            pltpu.VMEM((S, D), BF16),
            pltpu.VMEM((S, D), BF16),
            pltpu.VMEM((PADB + S, D), F32),
            pltpu.VMEM((8 + S + 8, D), F32),
            pltpu.VMEM((H, D // 2, E), U32), pltpu.VMEM((H, D // 2, E), U32), pltpu.VMEM((H, D // 2, E), U32),
            pltpu.VMEM((H * E // 2, D), U32),
            pltpu.VMEM((D, D), BF16), pltpu.VMEM((D, D), BF16), pltpu.VMEM((D, FF), BF16), pltpu.VMEM((FF, D), BF16),
            pltpu.VMEM((NST, 128, H, E), BF16),
            pltpu.VMEM((NST2, 512, D), BF16),
            pltpu.VMEM((M, D), BF16),
            pltpu.VMEM((24, D), U32),
            pltpu.VMEM((16, D), U32),
            pltpu.VMEM((3, 8, H * E), F32),
            pltpu.VMEM((8, H * E), F32),
            pltpu.VMEM((16, H * E), U32),
            pltpu.VMEM((24, H * E), U32),
            pltpu.VMEM((32, D), F32),
            pltpu.VMEM((48, D), F32),
            pltpu.VMEM((3, RB // 2, D), U32),
            pltpu.VMEM((RB, D), F32),
            pltpu.VMEM((RB // 2, FF), U32),
            pltpu.VMEM((PADB + S, D), BF16),
            pltpu.SemaphoreType.DMA((8 + NST + NST2,)),
        ],
        compiler_params=pltpu.CompilerParams(vmem_limit_bytes=120 * 1024 * 1024),
    )(x, mem0, wq, wk, wv, wo2, w1, w2, w3, w4)
```

```python
import functools

import jax
import jax.numpy as jnp
from jax.experimental import pallas as pl
from jax.experimental.pallas import tpu as pltpu

F32 = jnp.float32
BF16 = jnp.bfloat16
U32 = jnp.uint32
EPS = 1e-5


def _ln(x):
    m = jnp.mean(x, axis=-1, keepdims=True)
    xc = x - m
    v = jnp.mean(xc * xc, axis=-1, keepdims=True)
    return xc * jax.lax.rsqrt(v + EPS)


def _gelu(x):
    c = 0.7978845608028654
    return 0.5 * x * (1.0 + jnp.tanh(c * (x + 0.044715 * (x * x * x))))


def _dot(a, b):
    return jnp.dot(a, b, preferred_element_type=F32)


def _b(x):
    return pltpu.bitcast(x, BF16)


def _u(x):
    return pltpu.bitcast(x, U32)


def _mixer_schedule(H):
    s = {}

    def add(p, it, sl, op):
        s.setdefault((p, it, sl), []).append(op)

    def spread(ops, positions):
        assert len(ops) == len(positions), (len(ops), len(positions))
        for op, (p, it, sl) in zip(ops, positions):
            add(p, it, sl, op)

    def two(p, lo, hi):
        return [(p, it, sl) for it in range(lo, hi) for sl in (0, 1)]

    def tail(p):
        return [(p, H, 0)] * 3 + [(p, H + 1, 0)] * 2 + [(p, H + 2, 1)] * 4 + [(p, H + 3, 2)] * 4

    for c in range(4):
        add(1, c // 2, 2, ('ln1', c))
    spread([('w1', n, hf) for n in range(8) for hf in range(2)], two(1, 3, 11))
    for g in range(4):
        add(1, 6 + 2 * g, 2, ('mix', g))
    spread([('w2', n, 0) for n in range(8)], two(1, 11, 15))
    spread([('w2', n, 1) for n in range(8)], two(1, 15, 19))
    for c in range(4):
        add(1, 19 + c, 2, ('ln2', c))
    for p in (1, 2):
        add(p, 8, 2, ('prep',))
    w3 = [('w3', n, hf) for n in range(28) for hf in range(2)]
    pos3 = two(1, 23, H) + tail(1)
    pos3 = pos3 + two(2, 0, H)[:len(w3) - len(pos3)]
    spread(w3, pos3)
    first = (len([x for x in pos3 if x[0] == 2]) + 1) // 2 + 1
    w4 = [('w4', gi, n, pc) for gi in range(4) for n in range(8) for pc in range(2 if gi < 3 else 1)]
    its = list(range(first, H))
    extra = len(w4) - len(tail(2)) - 2 * len(its)
    pos4 = []
    for i, it in enumerate(its):
        pos4 += [(2, it, 0), (2, it, 1)] + ([(2, it, 2)] if i >= len(its) - extra else [])
    spread(w4, pos4 + tail(2))
    return s


def _make_kernel(S, D, H, E, M, SEG, FF):
    assert (SEG, M, E, H, D, FF) == (32, 8, 128, 32, 1024, 3584) and S == 2048
    NSEG = S // SEG
    NSUP = NSEG // 2
    RB = 2 * SEG
    TP = 24
    L0 = S - NSEG * TP
    R = 576
    ROFF = 64
    assert L0 == 512 and (L0 + ROFF) % R == 0 and R % (2 * TP) == 0 and R % SEG == 0
    scale = float(E) ** -0.5
    NT = D // 128
    NF = FF // 128
    PH = 8
    C4 = D // 4
    KH = D // 2
    HG = 8
    NG = H // HG
    HPI = 2
    NI = H // HPI
    PM = 128
    KS = 4
    PSKIP = 6
    G = 2
    LQ, LP = 2, 4
    sched = _mixer_schedule(H)

    def kernel(x_hbm, mem0_hbm, wq_hbm, wk_hbm, wv_hbm, wo_hbm, w1_hbm, w2_hbm, w3_hbm, w4_hbm,
               out_hbm,
               x_v, xn0_v, h_v, h1_v, wall_v, w1_v, w2_v, w3_v, w4_v,
               stage, stage2, mem_v, rq_v, rk_v, rv_v, lhs1_v, lhs2_v, tokb_v, os_v, o1_v, o2_v, acc1_v, acc2_v,
               bl_v, x1_v, t_v, out_v, zs, sems):
        srcs = [wq_hbm, wk_hbm, wv_hbm]
        rings = [rq_v, rk_v, rv_v]
        muls = [scale, None, None]
        S_X0, S_X1, S_MEM, S_B, S_OUT, S_ST, S_ST2 = 0, 1, 2, 3, 7, 8, 11

        cp_x0 = pltpu.make_async_copy(x_hbm.at[0, pl.ds(0, L0)], x_v.at[pl.ds(0, L0)], sems.at[S_X0])
        cp_m = pltpu.make_async_copy(mem0_hbm.at[0], mem_v, sems.at[S_MEM])

        def unit_cp(g, w):
            return pltpu.make_async_copy(srcs[w].at[:, pl.ds(pl.multiple_of(g * HG, HG), HG), :], stage.at[w],
                                         sems.at[S_ST + w])

        R2 = stage2.shape[1]

        def wo_cp(i):
            sl = jax.lax.rem(i, 2)
            return pltpu.make_async_copy(wo_hbm.at[pl.ds(pl.multiple_of(i * R2, R2), R2)], stage2.at[sl],
                                         sems.at[S_ST2 + sl])

        def chunks(src_ref, dst_ref, nrows, n, sem, row0=0):
            r = nrows // n
            return [pltpu.make_async_copy(src_ref.at[pl.ds(row0 + c * r, r)], dst_ref.at[pl.ds(row0 + c * r, r)], sem)
                    for c in range(n)]

        x1_cps = chunks(x_hbm.at[0], x_v, S - L0, 3, sems.at[S_X1], L0)
        w1_cps = chunks(w1_hbm, w1_v, D, 2, sems.at[S_B])
        w2_cps = chunks(w2_hbm, w2_v, D, 2, sems.at[S_B + 1])
        w3_cps = chunks(w3_hbm, w3_v, D, 4, sems.at[S_B + 2])
        w4_cps = chunks(w4_hbm, w4_v, FF, 2, sems.at[S_B + 3])
        extra = {3 + j: cp for j, cp in enumerate(x1_cps + w1_cps + w2_cps + w3_cps)}

        zs[0] = 0
        zs[1] = 0
        cp_x0.start()
        cp_m.start()
        for w in range(3):
            unit_cp(0, w).start()
        wo_cp(0).start()
        wo_cp(1).start()
        h1_v[pl.ds(0, PH), :] = jnp.zeros((PH, D), F32)
        h1_v[pl.ds(PH + S, PH), :] = jnp.zeros((PH, D), F32)
        cp_x0.wait()

        def ln_body(i, c):
            r0 = pl.multiple_of(i * 32, 32)
            xn0_v[pl.ds(pl.multiple_of(i * 16, 16), 16), :] = _u(_ln(x_v[pl.ds(r0, 32), :].astype(F32)).astype(BF16))
            return c
        jax.lax.fori_loop(0, L0 // 32, ln_body, 0)

        def relayout(g, w, t):
            v = stage[w, pl.ds(pl.multiple_of(t * 16, 16), 16)]
            wall_v[w + zs[0], pl.ds(pl.multiple_of(g * HG, HG), HG), pl.ds(pl.multiple_of(t * 8, 8), 8), :] = (
                _u(jnp.swapaxes(v, 0, 1)))

        NRL = D // 16
        for w in range(3):
            unit_cp(0, w).wait()

            def rl0(t, c, w=w):
                relayout(0, w, t)
                return c
            jax.lax.fori_loop(0, NRL, rl0, 0)
            if w < 2:
                unit_cp(1, w).start()

        NCV = R2 // 16
        IPG = HG // HPI

        def pro_body(i, c):
            g = i // IPG
            ii = jax.lax.rem(i, IPG)
            for w_ in range(3):
                @pl.when(jnp.logical_and(ii == w_ + 1, g + 1 < NG))
                def _(w_=w_):
                    unit_cp(g + 1, w_).wait()
            wo_cp(i).wait()
            gn = jnp.where(ii == 0, g, jnp.minimum(g + 1, NG - 1))
            wn = jnp.where(ii == 0, 2, ii - 1)
            sl2 = jax.lax.rem(i, 2)
            ND = HPI * 3 * (L0 // PM) * KS - PSKIP
            KW = D // KS
            n = 0
            for j in range(HPI):
                h = i * HPI + j
                for w in range(3):
                    for mb in range(L0 // PM):
                        y = None
                        for ks in range(KS):
                            yk = _dot(_b(xn0_v[pl.ds(mb * PM // 2, PM // 2), ks * KW:(ks + 1) * KW]),
                                      _b(wall_v[w + zs[1], h, pl.ds(ks * KW // 2, KW // 2), :]))
                            y = yk if y is None else y + yk
                            if ks == KS - 1:
                                if muls[w] is not None:
                                    y = y * muls[w]
                                rings[w][h, pl.ds(ROFF + mb * PM, PM), :] = y.astype(BF16)
                            for t in range(min(n, ND) * NRL // ND, min(n + 1, ND) * NRL // ND):
                                relayout(gn, wn, t)
                            for t in range(min(n, ND) * NCV // ND, min(n + 1, ND) * NCV // ND):
                                hh = i * HPI + t // (E // 16)
                                tr = (t % (E // 16)) * 8
                                cvt = _u(stage2[sl2, pl.ds(t * 16, 16), :])
                                for nn in range(NT):
                                    wall_v[3 + zs[0], hh, pl.ds(nn * (E // 2) + tr, 8), :] = (
                                        cvt[:, nn * 128:(nn + 1) * 128])
                            n += 1

            @pl.when(jnp.logical_and(ii == 0, g + 1 < NG))
            def _():
                unit_cp(g + 1, 2).start()

            @pl.when(jnp.logical_and(ii == 1, g + 2 < NG))
            def _():
                unit_cp(g + 2, 0).start()

            @pl.when(jnp.logical_and(ii == 2, g + 2 < NG))
            def _():
                unit_cp(g + 2, 1).start()

            @pl.when(i + 2 < NI)
            def _():
                wo_cp(i + 2).start()
            for it_, cp_ in extra.items():
                @pl.when(i == it_)
                def _(cp_=cp_):
                    cp_.start()
            return c
        jax.lax.fori_loop(0, NI, pro_body, 0)
        for cp in w4_cps:
            cp.start()
        cp_m.wait()
        for cp in x1_cps:
            cp.wait()

        P2 = 2 * SEG + 2 * M
        row = jax.lax.broadcasted_iota(jnp.int32, (P2, P2), 0)
        col = jax.lax.broadcasted_iota(jnp.int32, (P2, P2), 1)

        def head_of(z):
            return jnp.where(z < 2 * SEG, z // SEG, (z - 2 * SEG) // M)
        causal = jax.lax.rem(col, SEG) <= jax.lax.rem(row, SEG)
        allowed = (head_of(row) == head_of(col)) & ((row >= 2 * SEG) | (col >= 2 * SEG) | causal)

        def ln_tokens(t0):
            return _ln(x_v[pl.ds(pl.multiple_of(t0, 8), TP), :].astype(F32))

        def set_lhs(lhs_v, t0, mem):
            lhs_v[...] = _u(jnp.concatenate([ln_tokens(t0), mem], axis=0).astype(BF16))

        def prep_lhs(lhs_v, slot, t0):
            t = ln_tokens(t0)
            lhs_v[pl.ds(0, 8), :] = _u(t[0:16].astype(BF16))
            tokb_v[slot] = t[16:24]

        def finish_lhs(lhs_v, slot, mem):
            lhs_v[pl.ds(8, 8), :] = _u(jnp.concatenate([tokb_v[slot], mem], axis=0).astype(BF16))

        def b_ops(j1, j2):
            r1 = pl.multiple_of(j1 * RB, RB)
            r2 = pl.multiple_of(j2 * RB, RB)
            part = {}

            def half_dot(lhs_ref, w_ref, n, hf):
                return _dot(_b(lhs_ref[:, hf * KH:(hf + 1) * KH]),
                            w_ref[hf * KH:(hf + 1) * KH, n * 128:(n + 1) * 128])

            def ln1(c):
                a = _ln(_ln(h_v[pl.ds(r1 + 16 * c, 8), :]))
                b = _ln(_ln(h_v[pl.ds(r1 + 16 * c + 8, 8), :]))
                bl_v[0, pl.ds(8 * c, 8), :] = _u(jnp.concatenate([a, b], axis=0).astype(BF16))

            def w1(n, hf):
                y = half_dot(bl_v.at[0], w1_v, n, hf)
                if hf == 0:
                    part['w1'] = y
                else:
                    h1_v[pl.ds(r1 + PH, RB), n * 128:(n + 1) * 128] = _gelu(part.pop('w1') + y)

            def mix(g):
                off = (-1, 1, -2, 2)[g]
                win = h1_v[pl.ds(r2, RB + 2 * PH), g * C4:(g + 1) * C4]
                bl_v[1, :, g * C4:(g + 1) * C4] = _u(win[PH + off:PH + off + RB].astype(BF16))

            def w2(n, hf):
                y = half_dot(bl_v.at[1], w2_v, n, hf)
                if hf == 0:
                    x1_v[:, n * 128:(n + 1) * 128] = y
                else:
                    x1_v[:, n * 128:(n + 1) * 128] += y

            def ln2(c):
                res = []
                for hf in range(2):
                    rows = pl.ds(16 * c + 8 * hf, 8)
                    hb = h_v[pl.ds(r2 + 16 * c + 8 * hf, 8), :]
                    x1 = _ln(hb) + x1_v[rows, :]
                    x1_v[rows, :] = hb + x1
                    res.append(_ln(x1))
                bl_v[2, pl.ds(8 * c, 8), :] = _u(jnp.concatenate(res, axis=0).astype(BF16))

            def w3(n, hf):
                y = half_dot(bl_v.at[2], w3_v, n, hf)
                if hf == 0:
                    part['w3'] = y
                else:
                    t_v[:, n * 128:(n + 1) * 128] = _u(_gelu(part.pop('w3') + y).astype(BF16))

            def w4(gi, n, pc):
                k0 = gi * D + pc * KH
                y = _dot(_b(t_v[:, k0:k0 + KH]), w4_v[k0:k0 + KH, n * 128:(n + 1) * 128])
                if gi < 3 and pc == 0:
                    part['w4'] = y
                    return
                if gi < 3:
                    y = part.pop('w4') + y
                y = x1_v[:, n * 128:(n + 1) * 128] + y
                if gi < 3:
                    x1_v[:, n * 128:(n + 1) * 128] = y
                else:
                    out_v[pl.ds(r2, RB), n * 128:(n + 1) * 128] = y.astype(BF16)

            return dict(ln1=ln1, w1=w1, mix=mix, w2=w2, ln2=ln2, w3=w3, w4=w4)

        def phase(p, k, bops):
            lhs_v = lhs2_v if p == 2 else lhs1_v
            o_v = o1_v if p == 1 else o2_v
            acc_v = acc1_v if p == 1 else acc2_v
            if p == 0:
                wslot = pl.multiple_of(k * TP, 8)
                rbase = pl.multiple_of(k * SEG + ROFF, SEG)
            else:
                wbase = pl.multiple_of(jax.lax.rem(k * (2 * TP), R), 16)
                woff = 0 if p == 1 else TP
                rbase = pl.multiple_of(jax.lax.rem(k * RB + (p - 1) * SEG + ROFF, R), SEG)
            memf, pb, rinv, toks = {}, {}, {}, {}

            def proj(w, h):
                y = _dot(_b(lhs_v[...]), _b(wall_v[w, h]))
                if muls[w] is not None:
                    y = y * muls[w]
                if p == 0:
                    rings[w][h, pl.ds(wslot, TP), :] = y[0:TP].astype(BF16)
                else:
                    view = rings[w].at[h, pl.ds(wbase, 2 * TP)]
                    view[pl.ds(woff, TP), :] = y[0:TP].astype(BF16)
                memf[(w, h)] = y[TP:TP + M]

            def load_tok(w, j):
                toks[(w, j)] = [rings[w][2 * j + a, pl.ds(rbase, SEG), :] for a in range(2)]

            def full(w, j):
                mem16 = jnp.concatenate([memf.pop((w, 2 * j)), memf.pop((w, 2 * j + 1))], axis=0).astype(BF16)
                return jnp.concatenate(toks.pop((w, j)) + [mem16], axis=0)

            def qk(j):
                load_tok(1, j)
                sc = jax.lax.dot_general(full(0, j), full(1, j), (((1,), (1,)), ((), ())),
                                         preferred_element_type=F32)
                sc = jnp.where(allowed, sc, -1e30)
                pe = jnp.exp(sc - jnp.max(sc, axis=-1, keepdims=True))
                rinv[j] = pl.reciprocal(jnp.sum(pe, axis=-1, keepdims=True), approx=False)
                pb[j] = pe.astype(BF16)

            def pv(j):
                load_tok(2, j)
                o2 = _dot(pb.pop(j), full(2, j)) * rinv.pop(j)
                for a in range(2):
                    ot = o2[a * SEG:(a + 1) * SEG]
                    om = o2[2 * SEG + a * M:2 * SEG + (a + 1) * M]
                    cs = slice((2 * j + a) * E, (2 * j + a + 1) * E)
                    if p == 0:
                        o_v[:, cs] = _u(jnp.concatenate([ot, om, jnp.zeros((8, E), F32)], axis=0).astype(BF16))
                    elif p == 1:
                        o_v[:, cs] = _u(jnp.concatenate([ot[0:24], om], axis=0).astype(BF16))
                        os_v[:, cs] = ot[24:32]
                    else:
                        o_v[:, cs] = _u(jnp.concatenate([ot, om, os_v[:, cs]], axis=0).astype(BF16))

            def wo_group(g):
                ogs = [_b(o_v[:, (g * G + j) * E:(g * G + j + 1) * E]) for j in range(G)]
                for n in range(NT):
                    y = None
                    for j in range(G):
                        yj = _dot(ogs[j], _b(wall_v[3, g * G + j, pl.ds(n * (E // 2), E // 2), :]))
                        y = yj if y is None else y + yj
                    if g == 0:
                        acc_v[:, n * 128:(n + 1) * 128] = y
                    else:
                        acc_v[:, n * 128:(n + 1) * 128] += y

            def fin():
                if p == 0:
                    r0 = pl.multiple_of(k * SEG, SEG)
                    h_v[pl.ds(r0, SEG), :] = x_v[pl.ds(r0, SEG), :].astype(F32) + acc_v[pl.ds(0, SEG), :]
                    set_lhs(lhs1_v, L0 + (k + 1) * TP, acc_v[pl.ds(32, 8), :])
                    return
                r0 = pl.multiple_of(k * RB, RB)
                if p == 1:
                    h_v[pl.ds(r0, 24), :] = x_v[pl.ds(r0, 32), :].astype(F32)[0:24] + acc_v[pl.ds(0, 24), :]
                    finish_lhs(lhs2_v, 0, acc_v[pl.ds(24, 8), :])
                else:
                    xa = x_v[pl.ds(r0 + 16, 16), :].astype(F32)[8:16]
                    h_v[pl.ds(r0 + 24, 8), :] = xa + acc_v[pl.ds(40, 8), :]
                    h_v[pl.ds(r0 + 32, 32), :] = x_v[pl.ds(r0 + 32, 32), :].astype(F32) + acc_v[pl.ds(0, 32), :]
                    finish_lhs(lhs1_v, 1, acc_v[pl.ds(32, 8), :])

            def emit_b(it, sl):
                if bops is None:
                    return
                for op in sched.get((p, it, sl), []):
                    if op[0] == 'prep':
                        tnext = L0 + k * (2 * TP) + TP * p
                        if p == 1:
                            prep_lhs(lhs2_v, 0, tnext)
                        else:
                            prep_lhs(lhs1_v, 1, jnp.minimum(tnext, S - TP))
                    else:
                        bops[op[0]](*op[1:])

            NIT = H + LP
            for it in range(NIT):
                jq = (it - LQ) // 2 if (it - LQ) % 2 == 0 and 0 <= it - LQ < H else None
                jp = (it - LP) // 2 if (it - LP) % 2 == 0 and 0 <= it - LP < H else None
                if jq is not None:
                    load_tok(0, jq)
                if it < H:
                    proj(0, it)
                    emit_b(it, 0)
                if jq is not None:
                    qk(jq)
                if it >= H:
                    emit_b(it, 0)
                if it < H:
                    proj(1, it)
                    emit_b(it, 1)
                if jp is not None:
                    pv(jp)
                if it >= H:
                    emit_b(it, 1)
                if it < H:
                    proj(2, it)
                hd = it - LP
                if 0 <= hd < H and hd % G == G - 1:
                    wo_group(hd // G)
                if it == NIT - 1:
                    fin()
                emit_b(it, 2)

        def out_cp(j):
            r = pl.multiple_of(j * RB, RB)
            return pltpu.make_async_copy(out_v.at[pl.ds(r, RB)], out_hbm.at[0, pl.ds(r, RB)], sems.at[S_OUT])

        def run_ops(bops, names):
            for op in names:
                bops[op[0]](*op[1:])

        def a_body(s, c):
            phase(0, s, None)
            return c

        def sup_body(k, c):
            bops = b_ops(k - 1, k - 2)
            phase(1, k, bops)
            phase(2, k, bops)
            out_cp(k - 2).start()
            return c

        st1 = [('ln1', c) for c in range(4)] + [('w1', n, hf) for n in range(NT) for hf in range(2)]
        st2 = ([('mix', g) for g in range(4)] + [('w2', n, hf) for hf in range(2) for n in range(NT)]
               + [('ln2', c) for c in range(4)] + [('w3', n, hf) for n in range(NF) for hf in range(2)]
               + [('w4', gi, n, pc) for gi in range(4) for n in range(NT) for pc in range(2 if gi < 3 else 1)])

        set_lhs(lhs1_v, L0, mem_v[...].astype(F32))
        jax.lax.fori_loop(0, 4, a_body, 0)
        for cp in w1_cps:
            cp.wait()
        run_ops(b_ops(0, 0), st1)
        for cp in w2_cps + w3_cps + w4_cps:
            cp.wait()
        jax.lax.fori_loop(2, NSUP, sup_body, 0)

        run_ops(b_ops(NSUP - 1, NSUP - 1), st1)

        def epi_body(j, c):
            run_ops(b_ops(j, j), st2)
            out_cp(j).start()
            return c
        jax.lax.fori_loop(NSUP - 2, NSUP, epi_body, 0)
        for j in range(NSUP):
            out_cp(j).wait()

    scratch = [
        pltpu.VMEM((S, D), BF16),
        pltpu.VMEM((L0 // 2, D), U32),
        pltpu.VMEM((S, D), F32),
        pltpu.VMEM((PH + S + PH, D), F32),
        pltpu.VMEM((4, H, D // 2, E), U32),
        pltpu.VMEM((D, D), BF16), pltpu.VMEM((D, D), BF16), pltpu.VMEM((D, FF), BF16), pltpu.VMEM((FF, D), BF16),
        pltpu.VMEM((3, D, HG, E), BF16),
        pltpu.VMEM((2, HPI * E, D), BF16),
        pltpu.VMEM((M, D), BF16),
        pltpu.VMEM((H, R, E), BF16), pltpu.VMEM((H, R, E), BF16), pltpu.VMEM((H, R, E), BF16),
        pltpu.VMEM((16, D), U32),
        pltpu.VMEM((16, D), U32),
        pltpu.VMEM((2, 8, D), F32),
        pltpu.VMEM((8, H * E), F32),
        pltpu.VMEM((16, H * E), U32),
        pltpu.VMEM((24, H * E), U32),
        pltpu.VMEM((32, D), F32),
        pltpu.VMEM((48, D), F32),
        pltpu.VMEM((3, RB // 2, D), U32),
        pltpu.VMEM((RB, D), F32),
        pltpu.VMEM((RB // 2, FF), U32),
        pltpu.VMEM((S, D), BF16),
        pltpu.SMEM((2,), jnp.int32),
        pltpu.SemaphoreType.DMA((13,)),
    ]
    return kernel, scratch


@functools.partial(jax.jit, static_argnames=("A_seg_len",))
def pallas_sequential_preLN__memory_aug_recurrent_mem_tr__mixer_s_mlp__prompt_kernel(
        A_x, A_mem0, A_Wq, A_Wk, A_Wv, A_Wo, A_seg_len, B_x, B_w1, B_w2, B_w3, B_w4):
    del B_x
    B, S, D = A_x.shape
    _, H, E = A_Wq.shape
    assert B == 1
    kernel, scratch = _make_kernel(S, D, H, E, A_mem0.shape[1], int(A_seg_len), B_w3.shape[1])
    any_spec = pl.BlockSpec(memory_space=pl.ANY)
    return pl.pallas_call(
        kernel,
        out_shape=jax.ShapeDtypeStruct((B, S, D), BF16),
        in_specs=[any_spec] * 10,
        out_specs=any_spec,
        scratch_shapes=scratch,
        compiler_params=pltpu.CompilerParams(vmem_limit_bytes=120 * 1024 * 1024),
    )(A_x, A_mem0, A_Wq, A_Wk, A_Wv, A_Wo.reshape(H * E, D), B_w1, B_w2, B_w3, B_w4)
```

```python
import functools

import jax
import jax.numpy as jnp
from jax.experimental import pallas as pl
from jax.experimental.pallas import tpu as pltpu

F32 = jnp.float32
BF16 = jnp.bfloat16
U32 = jnp.uint32
EPS = 1e-5


def _ln(x):
    m = jnp.mean(x, axis=-1, keepdims=True)
    xc = x - m
    v = jnp.mean(xc * xc, axis=-1, keepdims=True)
    return xc * jax.lax.rsqrt(v + EPS)


def _gelu(x):
    c = 0.7978845608028654
    return 0.5 * x * (1.0 + jnp.tanh(c * (x + 0.044715 * (x * x * x))))


def _dot(a, b):
    return jnp.dot(a, b, preferred_element_type=F32)


def _b(x):
    return pltpu.bitcast(x, BF16)


def _u(x):
    return pltpu.bitcast(x, U32)


def _mixer_schedule(H):
    s = {}

    def add(p, it, sl, op):
        s.setdefault((p, it, sl), []).append(op)

    def spread(ops, positions):
        assert len(ops) == len(positions), (len(ops), len(positions))
        for op, (p, it, sl) in zip(ops, positions):
            add(p, it, sl, op)

    def two(p, lo, hi):
        return [(p, it, sl) for it in range(lo, hi) for sl in (0, 1)]

    def tail(p):
        return [(p, H, 0)] * 3 + [(p, H + 1, 0)] * 2 + [(p, H + 2, 1)] * 4 + [(p, H + 3, 2)] * 4

    for c in range(4):
        add(1, c // 2, 2, ('ln1', c))
    spread([('w1', n, hf) for n in range(8) for hf in range(2)], two(1, 3, 11))
    for g in range(4):
        add(1, 6 + 2 * g, 2, ('mix', g))
    spread([('w2', n, 0) for n in range(8)], two(1, 11, 15))
    spread([('w2', n, 1) for n in range(8)], two(1, 15, 19))
    for c in range(4):
        add(1, 19 + c, 2, ('ln2', c))
    for p in (1, 2):
        add(p, 8, 2, ('prep',))
    w3 = [('w3', n, hf) for n in range(28) for hf in range(2)]
    pos3 = two(1, 23, H) + tail(1)
    pos3 = pos3 + two(2, 0, H)[:len(w3) - len(pos3)]
    spread(w3, pos3)
    first = (len([x for x in pos3 if x[0] == 2]) + 1) // 2 + 1
    w4 = [('w4', gi, n, pc) for gi in range(4) for n in range(8) for pc in range(2 if gi < 3 else 1)]
    its = list(range(first, H))
    extra = len(w4) - len(tail(2)) - 2 * len(its)
    pos4 = []
    for i, it in enumerate(its):
        pos4 += [(2, it, 0), (2, it, 1)] + ([(2, it, 2)] if i >= len(its) - extra else [])
    spread(w4, pos4 + tail(2))
    return s


def _make_kernel(S, D, H, E, M, SEG, FF):
    assert (SEG, M, E, H, D, FF) == (32, 8, 128, 32, 1024, 3584) and S == 2048
    NSEG = S // SEG
    NSUP = NSEG // 2
    RB = 2 * SEG
    TP = 24
    L0 = S - NSEG * TP
    R = 576
    ROFF = 64
    assert L0 == 512 and (L0 + ROFF) % R == 0 and R % (2 * TP) == 0 and R % SEG == 0
    scale = float(E) ** -0.5
    NT = D // 128
    NF = FF // 128
    PH = 8
    C4 = D // 4
    KH = D // 2
    HG = 8
    NG = H // HG
    PM = 128
    KS = 4
    PSKIP = 6
    G = 2
    LQ, LP = 2, 4
    sched = _mixer_schedule(H)

    def kernel(x_hbm, mem0_hbm, wq_hbm, wk_hbm, wv_hbm, wo_hbm, w1_hbm, w2_hbm, w3_hbm, w4_hbm,
               out_hbm,
               x_v, xn0_v, h_v, h1_v, wall_v, w1_v, w2_v, w3_v, w4_v,
               stage, stage2, mem_v, rq_v, rk_v, rv_v, lhs1_v, lhs2_v, tokb_v, os_v, o1_v, o2_v, acc1_v, acc2_v,
               bl_v, x1_v, t_v, out_v, zs, sems):
        srcs = [wq_hbm, wk_hbm, wv_hbm]
        rings = [rq_v, rk_v, rv_v]
        muls = [scale, None, None]
        S_X0, S_X1, S_MEM, S_B, S_OUT, S_ST, S_ST2 = 0, 1, 2, 3, 7, 8, 11

        cp_x0 = pltpu.make_async_copy(x_hbm.at[0, pl.ds(0, L0)], x_v.at[pl.ds(0, L0)], sems.at[S_X0])
        cp_m = pltpu.make_async_copy(mem0_hbm.at[0], mem_v, sems.at[S_MEM])

        def unit_cp(g, w):
            return pltpu.make_async_copy(srcs[w].at[:, pl.ds(pl.multiple_of(g * HG, HG), HG), :], stage.at[w],
                                         sems.at[S_ST + w])

        R2 = stage2.shape[1]

        NCV = R2 // 16
        NCH = H * E // 16

        def wo_cp(i):
            sl = jax.lax.rem(i, 2)
            r0 = pl.multiple_of(jnp.minimum(i * R2, H * E - R2), 16)
            return pltpu.make_async_copy(wo_hbm.at[pl.ds(r0, R2)], stage2.at[sl], sems.at[S_ST2 + sl])

        def chunks(src_ref, dst_ref, nrows, n, sem, row0=0):
            r = nrows // n
            return [pltpu.make_async_copy(src_ref.at[pl.ds(row0 + c * r, r)], dst_ref.at[pl.ds(row0 + c * r, r)], sem)
                    for c in range(n)]

        x1_cps = chunks(x_hbm.at[0], x_v, S - L0, 3, sems.at[S_X1], L0)
        w1_cps = chunks(w1_hbm, w1_v, D, 2, sems.at[S_B])
        w2_cps = chunks(w2_hbm, w2_v, D, 2, sems.at[S_B + 1])
        w3_cps = chunks(w3_hbm, w3_v, D, 4, sems.at[S_B + 2])
        w4_cps = chunks(w4_hbm, w4_v, FF, 2, sems.at[S_B + 3])
        extra = {2 + j: cp for j, cp in enumerate(x1_cps + w1_cps + w2_cps + w3_cps[:2])}
        late = w3_cps[2:] + w4_cps

        zs[0] = 0
        zs[1] = 0
        cp_x0.start()
        cp_m.start()
        for w in range(3):
            unit_cp(0, w).start()
        wo_cp(0).start()
        stage2[1] = jnp.zeros(stage2.shape[1:], BF16)
        h1_v[pl.ds(0, PH), :] = jnp.zeros((PH, D), F32)
        h1_v[pl.ds(PH + S, PH), :] = jnp.zeros((PH, D), F32)
        cp_x0.wait()

        def ln_body(i, c):
            r0 = pl.multiple_of(i * 32, 32)
            xn0_v[pl.ds(pl.multiple_of(i * 16, 16), 16), :] = _u(_ln(x_v[pl.ds(r0, 32), :].astype(F32)).astype(BF16))
            return c
        jax.lax.fori_loop(0, L0 // 32, ln_body, 0)

        def relayout(g, w, t):
            v = stage[w, pl.ds(pl.multiple_of(t * 16, 16), 16)]
            wall_v[w + zs[0], pl.ds(pl.multiple_of(g * HG, HG), HG), pl.ds(pl.multiple_of(t * 8, 8), 8), :] = (
                _u(jnp.swapaxes(v, 0, 1)))

        NRL = D // 16
        unit_cp(0, 0).wait()

        def rl0(t, c):
            for u in range(4):
                relayout(0, 0, t * 4 + u)
            return c
        jax.lax.fori_loop(0, NRL // 4, rl0, 0)
        unit_cp(1, 0).start()

        NU = 3 * NG

        def pro_body(u, c):
            g = u // 3
            w = jax.lax.rem(u, 3)
            un = jnp.where(u + 1 < NU, u + 1, NU - 3)
            gn = un // 3
            wn = jax.lax.rem(un, 3)
            sl2 = jax.lax.rem(u + 1, 2)
            c0 = jnp.clip((u - 1) * NCV, 0, NCH - NCV)
            mul = jnp.where(w == 0, scale, 1.0).astype(F32)
            wvec = jnp.full((PM // 2, E), w, jnp.int32)
            msk = [wvec == w_ for w_ in range(3)]

            for w_ in range(3):
                @pl.when(jnp.logical_and(wn == w_, u + 1 < NU))
                def _(w_=w_):
                    unit_cp(gn, w_).wait()

            @pl.when(u >= 1)
            def _():
                wo_cp(u - 1).wait()
            ND = HG * (L0 // PM) * KS - PSKIP
            KW = D // KS
            n = 0
            for j in range(HG):
                h = g * HG + j
                for mb in range(L0 // PM):
                    y = None
                    for ks in range(KS):
                        yk = _dot(_b(xn0_v[pl.ds(mb * PM // 2, PM // 2), ks * KW:(ks + 1) * KW]),
                                  _b(wall_v[w + zs[1], h, pl.ds(ks * KW // 2, KW // 2), :]))
                        y = yk if y is None else y + yk
                        if ks == KS - 1:
                            yb = _u((y * mul).astype(BF16))
                            for w_ in range(3):
                                pltpu.store(rings[w_].at[h, pl.ds((ROFF + mb * PM) // 2, PM // 2), :], yb,
                                            mask=msk[w_])
                        for t in range(min(n, ND) * NRL // ND, min(n + 1, ND) * NRL // ND):
                            relayout(gn, wn, t)
                        for t in range(min(n, ND) * NCV // ND, min(n + 1, ND) * NCV // ND):
                            ch = c0 + t
                            hh = ch // (E // 16)
                            tr = pl.multiple_of(jax.lax.rem(ch, E // 16) * 8, 8)
                            cvt = _u(stage2[sl2, pl.ds(t * 16, 16), :])
                            for nn in range(NT):
                                wall_v[3 + zs[0], hh, pl.ds(nn * (E // 2) + tr, 8), :] = (
                                    cvt[:, nn * 128:(nn + 1) * 128])
                        n += 1

            @pl.when(u + 1 < NWO)
            def _():
                wo_cp(u + 1).start()
            for w_ in range(3):
                @pl.when(jnp.logical_and(wn == w_, u + 4 < NU))
                def _(w_=w_):
                    unit_cp(gn + 1, w_).start()
            for it_, cp_ in extra.items():
                @pl.when(u == it_)
                def _(cp_=cp_):
                    cp_.start()
            return c
        NWO = -(-NCH // NCV)
        assert NWO == NU - 1
        jax.lax.fori_loop(0, NU, pro_body, 0)
        for cp in late:
            cp.start()
        cp_m.wait()
        for cp in x1_cps:
            cp.wait()

        P2 = 2 * SEG + 2 * M
        row = jax.lax.broadcasted_iota(jnp.int32, (P2, P2), 0)
        col = jax.lax.broadcasted_iota(jnp.int32, (P2, P2), 1)

        def head_of(z):
            return jnp.where(z < 2 * SEG, z // SEG, (z - 2 * SEG) // M)
        causal = jax.lax.rem(col, SEG) <= jax.lax.rem(row, SEG)
        allowed = (head_of(row) == head_of(col)) & ((row >= 2 * SEG) | (col >= 2 * SEG) | causal)

        def ln_tokens(t0):
            return _ln(x_v[pl.ds(pl.multiple_of(t0, 8), TP), :].astype(F32))

        def set_lhs(lhs_v, t0, mem):
            lhs_v[...] = _u(jnp.concatenate([ln_tokens(t0), mem], axis=0).astype(BF16))

        def prep_lhs(lhs_v, slot, t0):
            t = ln_tokens(t0)
            lhs_v[pl.ds(0, 8), :] = _u(t[0:16].astype(BF16))
            tokb_v[slot] = t[16:24]

        def finish_lhs(lhs_v, slot, mem):
            lhs_v[pl.ds(8, 8), :] = _u(jnp.concatenate([tokb_v[slot], mem], axis=0).astype(BF16))

        def b_ops(j1, j2):
            r1 = pl.multiple_of(j1 * RB, RB)
            r2 = pl.multiple_of(j2 * RB, RB)
            part = {}

            def half_dot(lhs_ref, w_ref, n, hf):
                return _dot(_b(lhs_ref[:, hf * KH:(hf + 1) * KH]),
                            w_ref[hf * KH:(hf + 1) * KH, n * 128:(n + 1) * 128])

            def ln1(c):
                a = _ln(_ln(h_v[pl.ds(r1 + 16 * c, 8), :]))
                b = _ln(_ln(h_v[pl.ds(r1 + 16 * c + 8, 8), :]))
                bl_v[0, pl.ds(8 * c, 8), :] = _u(jnp.concatenate([a, b], axis=0).astype(BF16))

            def w1(n, hf):
                y = half_dot(bl_v.at[0], w1_v, n, hf)
                if hf == 0:
                    part['w1'] = y
                else:
                    h1_v[pl.ds(r1 + PH, RB), n * 128:(n + 1) * 128] = _gelu(part.pop('w1') + y)

            def mix(g):
                off = (-1, 1, -2, 2)[g]
                win = h1_v[pl.ds(r2, RB + 2 * PH), g * C4:(g + 1) * C4]
                bl_v[1, :, g * C4:(g + 1) * C4] = _u(win[PH + off:PH + off + RB].astype(BF16))

            def w2(n, hf):
                y = half_dot(bl_v.at[1], w2_v, n, hf)
                if hf == 0:
                    x1_v[:, n * 128:(n + 1) * 128] = y
                else:
                    x1_v[:, n * 128:(n + 1) * 128] += y

            def ln2(c):
                res = []
                for hf in range(2):
                    rows = pl.ds(16 * c + 8 * hf, 8)
                    hb = h_v[pl.ds(r2 + 16 * c + 8 * hf, 8), :]
                    x1 = _ln(hb) + x1_v[rows, :]
                    x1_v[rows, :] = hb + x1
                    res.append(_ln(x1))
                bl_v[2, pl.ds(8 * c, 8), :] = _u(jnp.concatenate(res, axis=0).astype(BF16))

            def w3(n, hf):
                y = half_dot(bl_v.at[2], w3_v, n, hf)
                if hf == 0:
                    part['w3'] = y
                else:
                    t_v[:, n * 128:(n + 1) * 128] = _u(_gelu(part.pop('w3') + y).astype(BF16))

            def w4(gi, n, pc):
                k0 = gi * D + pc * KH
                y = _dot(_b(t_v[:, k0:k0 + KH]), w4_v[k0:k0 + KH, n * 128:(n + 1) * 128])
                if gi < 3 and pc == 0:
                    part['w4'] = y
                    return
                if gi < 3:
                    y = part.pop('w4') + y
                y = x1_v[:, n * 128:(n + 1) * 128] + y
                if gi < 3:
                    x1_v[:, n * 128:(n + 1) * 128] = y
                else:
                    out_v[pl.ds(r2, RB), n * 128:(n + 1) * 128] = y.astype(BF16)

            return dict(ln1=ln1, w1=w1, mix=mix, w2=w2, ln2=ln2, w3=w3, w4=w4)

        def phase(p, k, bops):
            lhs_v = lhs2_v if p == 2 else lhs1_v
            o_v = o1_v if p == 1 else o2_v
            acc_v = acc1_v if p == 1 else acc2_v
            if p == 0:
                odd = jax.lax.rem(k, 2)
                wbase = pl.multiple_of((k // 2) * TP, 8)
                rbase = pl.multiple_of(k * (SEG // 2) + ROFF // 2, SEG // 2)
                keep_new = jax.lax.broadcasted_iota(jnp.int32, (8, E), 0) // 4 == odd
            else:
                wbase = pl.multiple_of(jax.lax.rem(k * TP, R // 2), 8)
                rbase = pl.multiple_of(jax.lax.rem(k * SEG + (p - 1) * (SEG // 2) + ROFF // 2, R // 2), SEG // 2)
            memf, pb, rinv, toks = {}, {}, {}, {}

            def proj(w, h):
                y = _dot(_b(lhs_v[...]), _b(wall_v[w, h]))
                if muls[w] is not None:
                    y = y * muls[w]
                view = rings[w].at[h, pl.ds(wbase, TP)]
                if p == 1:
                    view[pl.ds(0, 8), :] = _u(y[0:16].astype(BF16))
                    view[pl.ds(8, 4), :] = _u(y[16:32].astype(BF16))[0:4]
                elif p == 2:
                    view[pl.ds(12, 4), :] = _u(jnp.concatenate([y[0:8], y[0:8]], axis=0).astype(BF16))[4:8]
                    view[pl.ds(16, 8), :] = _u(y[8:24].astype(BF16))
                else:
                    is_odd = odd == 1
                    fullv = jnp.where(is_odd, _u(y[8:24].astype(BF16)), _u(y[0:16].astype(BF16)))
                    halfv = jnp.where(is_odd, _u(jnp.concatenate([y[0:8], y[0:8]], axis=0).astype(BF16)),
                                      _u(y[16:32].astype(BF16)))
                    view[pl.ds(pl.multiple_of(odd * 16, 8), 8), :] = fullv
                    view[pl.ds(8, 8), :] = jnp.where(keep_new, halfv, view[pl.ds(8, 8), :])
                memf[(w, h)] = y[TP:TP + M]

            def load_tok(w, j):
                toks[(w, j)] = [_b(rings[w][2 * j + a, pl.ds(rbase, SEG // 2), :]) for a in range(2)]

            def full(w, j):
                mem16 = jnp.concatenate([memf.pop((w, 2 * j)), memf.pop((w, 2 * j + 1))], axis=0).astype(BF16)
                return jnp.concatenate(toks.pop((w, j)) + [mem16], axis=0)

            def qk(j):
                load_tok(1, j)
                sc = jax.lax.dot_general(full(0, j), full(1, j), (((1,), (1,)), ((), ())),
                                         preferred_element_type=F32)
                sc = jnp.where(allowed, sc, -1e30)
                pe = jnp.exp(sc - jnp.max(sc, axis=-1, keepdims=True))
                rinv[j] = pl.reciprocal(jnp.sum(pe, axis=-1, keepdims=True), approx=False)
                pb[j] = pe.astype(BF16)

            def pv(j):
                load_tok(2, j)
                o2 = _dot(pb.pop(j), full(2, j)) * rinv.pop(j)
                for a in range(2):
                    ot = o2[a * SEG:(a + 1) * SEG]
                    om = o2[2 * SEG + a * M:2 * SEG + (a + 1) * M]
                    cs = slice((2 * j + a) * E, (2 * j + a + 1) * E)
                    if p == 0:
                        o_v[:, cs] = _u(jnp.concatenate([ot, om, jnp.zeros((8, E), F32)], axis=0).astype(BF16))
                    elif p == 1:
                        o_v[:, cs] = _u(jnp.concatenate([ot[0:24], om], axis=0).astype(BF16))
                        os_v[:, cs] = ot[24:32]
                    else:
                        o_v[:, cs] = _u(jnp.concatenate([ot, om, os_v[:, cs]], axis=0).astype(BF16))

            def wo_group(g):
                ogs = [_b(o_v[:, (g * G + j) * E:(g * G + j + 1) * E]) for j in range(G)]
                for n in range(NT):
                    y = None
                    for j in range(G):
                        yj = _dot(ogs[j], _b(wall_v[3, g * G + j, pl.ds(n * (E // 2), E // 2), :]))
                        y = yj if y is None else y + yj
                    if g == 0:
                        acc_v[:, n * 128:(n + 1) * 128] = y
                    else:
                        acc_v[:, n * 128:(n + 1) * 128] += y

            def fin():
                if p == 0:
                    r0 = pl.multiple_of(k * SEG, SEG)
                    h_v[pl.ds(r0, SEG), :] = x_v[pl.ds(r0, SEG), :].astype(F32) + acc_v[pl.ds(0, SEG), :]
                    set_lhs(lhs1_v, L0 + (k + 1) * TP, acc_v[pl.ds(32, 8), :])
                    return
                r0 = pl.multiple_of(k * RB, RB)
                if p == 1:
                    h_v[pl.ds(r0, 24), :] = x_v[pl.ds(r0, 32), :].astype(F32)[0:24] + acc_v[pl.ds(0, 24), :]
                    finish_lhs(lhs2_v, 0, acc_v[pl.ds(24, 8), :])
                else:
                    xa = x_v[pl.ds(r0 + 16, 16), :].astype(F32)[8:16]
                    h_v[pl.ds(r0 + 24, 8), :] = xa + acc_v[pl.ds(40, 8), :]
                    h_v[pl.ds(r0 + 32, 32), :] = x_v[pl.ds(r0 + 32, 32), :].astype(F32) + acc_v[pl.ds(0, 32), :]
                    finish_lhs(lhs1_v, 1, acc_v[pl.ds(32, 8), :])

            def emit_b(it, sl):
                if bops is None:
                    return
                for op in sched.get((p, it, sl), []):
                    if op[0] == 'prep':
                        tnext = L0 + k * (2 * TP) + TP * p
                        if p == 1:
                            prep_lhs(lhs2_v, 0, tnext)
                        else:
                            prep_lhs(lhs1_v, 1, jnp.minimum(tnext, S - TP))
                    else:
                        bops[op[0]](*op[1:])

            NIT = H + LP
            for it in range(NIT):
                jq = (it - LQ) // 2 if (it - LQ) % 2 == 0 and 0 <= it - LQ < H else None
                jp = (it - LP) // 2 if (it - LP) % 2 == 0 and 0 <= it - LP < H else None
                if jq is not None:
                    load_tok(0, jq)
                if it < H:
                    proj(0, it)
                    emit_b(it, 0)
                if jq is not None:
                    qk(jq)
                if it >= H:
                    emit_b(it, 0)
                if it < H:
                    proj(1, it)
                    emit_b(it, 1)
                if jp is not None:
                    pv(jp)
                if it >= H:
                    emit_b(it, 1)
                if it < H:
                    proj(2, it)
                hd = it - LP
                if 0 <= hd < H and hd % G == G - 1:
                    wo_group(hd // G)
                if it == NIT - 1:
                    fin()
                emit_b(it, 2)

        def out_cp(j):
            r = pl.multiple_of(j * RB, RB)
            return pltpu.make_async_copy(out_v.at[pl.ds(r, RB)], out_hbm.at[0, pl.ds(r, RB)], sems.at[S_OUT])

        def run_ops(bops, names):
            for op in names:
                bops[op[0]](*op[1:])

        def a_body(s, c):
            phase(0, s, None)
            return c

        def sup_body(k, c):
            bops = b_ops(k - 1, k - 2)
            phase(1, k, bops)
            phase(2, k, bops)
            out_cp(k - 2).start()
            return c

        st1 = [('ln1', c) for c in range(4)] + [('w1', n, hf) for n in range(NT) for hf in range(2)]
        st2 = ([('mix', g) for g in range(4)] + [('w2', n, hf) for hf in range(2) for n in range(NT)]
               + [('ln2', c) for c in range(4)] + [('w3', n, hf) for n in range(NF) for hf in range(2)]
               + [('w4', gi, n, pc) for gi in range(4) for n in range(NT) for pc in range(2 if gi < 3 else 1)])

        set_lhs(lhs1_v, L0, mem_v[...].astype(F32))
        jax.lax.fori_loop(0, 4, a_body, 0)
        for cp in w1_cps:
            cp.wait()
        run_ops(b_ops(0, 0), st1)
        for cp in w2_cps + w3_cps + w4_cps:
            cp.wait()
        jax.lax.fori_loop(2, NSUP, sup_body, 0)

        run_ops(b_ops(NSUP - 1, NSUP - 1), st1)

        def epi_body(j, c):
            run_ops(b_ops(j, j), st2)
            out_cp(j).start()
            return c
        jax.lax.fori_loop(NSUP - 2, NSUP, epi_body, 0)
        for j in range(NSUP):
            out_cp(j).wait()

    scratch = [
        pltpu.VMEM((S, D), BF16),
        pltpu.VMEM((L0 // 2, D), U32),
        pltpu.VMEM((S, D), F32),
        pltpu.VMEM((PH + S + PH, D), F32),
        pltpu.VMEM((4, H, D // 2, E), U32),
        pltpu.VMEM((D, D), BF16), pltpu.VMEM((D, D), BF16), pltpu.VMEM((D, FF), BF16), pltpu.VMEM((FF, D), BF16),
        pltpu.VMEM((3, D, HG, E), BF16),
        pltpu.VMEM((2, 384, D), BF16),
        pltpu.VMEM((M, D), BF16),
        pltpu.VMEM((H, R // 2, E), U32), pltpu.VMEM((H, R // 2, E), U32), pltpu.VMEM((H, R // 2, E), U32),
        pltpu.VMEM((16, D), U32),
        pltpu.VMEM((16, D), U32),
        pltpu.VMEM((2, 8, D), F32),
        pltpu.VMEM((8, H * E), F32),
        pltpu.VMEM((16, H * E), U32),
        pltpu.VMEM((24, H * E), U32),
        pltpu.VMEM((32, D), F32),
        pltpu.VMEM((48, D), F32),
        pltpu.VMEM((3, RB // 2, D), U32),
        pltpu.VMEM((RB, D), F32),
        pltpu.VMEM((RB // 2, FF), U32),
        pltpu.VMEM((S, D), BF16),
        pltpu.SMEM((2,), jnp.int32),
        pltpu.SemaphoreType.DMA((13,)),
    ]
    return kernel, scratch


@functools.partial(jax.jit, static_argnames=("A_seg_len",))
def pallas_sequential_preLN__memory_aug_recurrent_mem_tr__mixer_s_mlp__prompt_kernel(
        A_x, A_mem0, A_Wq, A_Wk, A_Wv, A_Wo, A_seg_len, B_x, B_w1, B_w2, B_w3, B_w4):
    del B_x
    B, S, D = A_x.shape
    _, H, E = A_Wq.shape
    assert B == 1
    kernel, scratch = _make_kernel(S, D, H, E, A_mem0.shape[1], int(A_seg_len), B_w3.shape[1])
    any_spec = pl.BlockSpec(memory_space=pl.ANY)
    return pl.pallas_call(
        kernel,
        out_shape=jax.ShapeDtypeStruct((B, S, D), BF16),
        in_specs=[any_spec] * 10,
        out_specs=any_spec,
        scratch_shapes=scratch,
        compiler_params=pltpu.CompilerParams(vmem_limit_bytes=120 * 1024 * 1024, disable_bounds_checks=True),
    )(A_x, A_mem0, A_Wq, A_Wk, A_Wv, A_Wo.reshape(H * E, D), B_w1, B_w2, B_w3, B_w4)
```

```python
import functools

import jax
import jax.numpy as jnp
from jax.experimental import pallas as pl
from jax.experimental.pallas import tpu as pltpu

F32 = jnp.float32
BF16 = jnp.bfloat16
U32 = jnp.uint32
EPS = 1e-5


def _ln(x):
    m = jnp.mean(x, axis=-1, keepdims=True)
    xc = x - m
    v = jnp.mean(xc * xc, axis=-1, keepdims=True)
    return xc * jax.lax.rsqrt(v + EPS)


def _gelu(x):
    c = 0.7978845608028654
    return 0.5 * x * (1.0 + jnp.tanh(c * (x + 0.044715 * (x * x * x))))


def _dot(a, b):
    return jnp.dot(a, b, preferred_element_type=F32)


def _b(x):
    return pltpu.bitcast(x, BF16)


def _u(x):
    return pltpu.bitcast(x, U32)


def _mixer_schedule(H):
    s = {}

    def add(p, it, sl, op):
        s.setdefault((p, it, sl), []).append(op)

    def spread(ops, positions):
        assert len(ops) == len(positions), (len(ops), len(positions))
        for op, (p, it, sl) in zip(ops, positions):
            add(p, it, sl, op)

    def two(p, lo, hi):
        return [(p, it, sl) for it in range(lo, hi) for sl in (0, 1)]

    def tail(p):
        return [(p, H, 0)] * 3 + [(p, H + 1, 0)] * 2 + [(p, H + 2, 1)] * 4 + [(p, H + 3, 2)] * 4

    add(1, 0, 0, ('mix', 0))
    add(1, 0, 0, ('mix', 2))
    for c in range(4):
        add(1, c // 2, 2, ('ln1', c))
    spread([('w2', n, 0) for n in range(8)], two(1, 1, 5))
    spread([('w1', n, hf) for n in range(8) for hf in range(2)], two(1, 5, 13))
    add(1, 10, 2, ('mix', 1))
    add(1, 15, 2, ('mix', 3))
    spread([('w2', n, 1) for n in range(8)], two(1, 16, 20))
    for c in range(4):
        add(1, 20 + c, 2, ('ln2', c))
    for p in (1, 2):
        add(p, 8, 2, ('prep',))
    w3 = [('w3', n, hf) for n in range(28) for hf in range(2)]
    pos3 = two(1, 24, H) + tail(1)
    pos3 = pos3 + two(2, 0, H)[:len(w3) - len(pos3)]
    spread(w3, pos3)
    first = max(x[1] for x in pos3 if x[0] == 2) + 2
    w4 = [('w4', gi, n, pc) for gi in range(4) for n in range(8) for pc in range(2 if gi < 3 else 1)]
    its = list(range(first, H))
    extra = len(w4) - len(tail(2)) - 2 * len(its)
    pos4 = []
    for i, it in enumerate(its):
        pos4 += [(2, it, 0), (2, it, 1)] + ([(2, it, 2)] if i >= len(its) - extra else [])
    spread(w4, pos4 + tail(2))

    slot_order = {0: 0, 1: 1, 2: 2}
    seq = [op for key in sorted(s, key=lambda k: (k[0], k[1], slot_order[k[2]])) for op in s[key]]
    pos = {op: i for i, op in enumerate(seq)}
    last = lambda name: max(i for op, i in pos.items() if op[0] == name)
    first_ = lambda name: min(i for op, i in pos.items() if op[0] == name)
    assert last('ln1') < first_('w1') and last('w2') < first_('ln2') and last('ln2') < first_('w3')
    assert pos[('w1', 3, 1)] < pos[('mix', 1)] and pos[('w1', 7, 1)] < pos[('mix', 3)]
    assert max(pos[('mix', 0)], pos[('mix', 2)]) < min(pos[('w2', n, 0)] for n in range(8))
    assert max(pos[('mix', 1)], pos[('mix', 3)]) < min(pos[('w2', n, 1)] for n in range(8))
    assert all(pos[('w2', n, 0)] < pos[('w2', n, 1)] for n in range(8))
    for gi in range(4):
        assert pos[('w3', min(8 * gi + 7, 27), 1)] < min(i for op, i in pos.items() if op[0] == 'w4' and op[1] == gi)
    return s


def _make_kernel(S, D, H, E, M, SEG, FF):
    assert (SEG, M, E, H, D, FF) == (32, 8, 128, 32, 1024, 3584) and S == 2048
    NSEG = S // SEG
    NSUP = NSEG // 2
    RB = 2 * SEG
    TP = 24
    L0 = S - NSEG * TP
    R = 576
    ROFF = 64
    assert L0 == 512 and (L0 + ROFF) % R == 0 and R % (2 * TP) == 0 and R % SEG == 0
    scale = float(E) ** -0.5
    NT = D // 128
    NF = FF // 128
    PH = 8
    C4 = D // 4
    KH = D // 2
    HG = 8
    NG = H // HG
    PM = 128
    KS = 4
    PSKIP = 6
    G = 2
    LQ, LP = 2, 4
    sched = _mixer_schedule(H)

    def kernel(x_hbm, mem0_hbm, wq_hbm, wk_hbm, wv_hbm, wo_hbm, w1_hbm, w2_hbm, w3_hbm, w4_hbm,
               out_hbm,
               x_v, xn0_v, h_v, h1_v, wall_v, w1_v, w2_v, w3_v, w4_v,
               stage, stage2, mem_v, rq_v, rk_v, rv_v, lhs1_v, lhs2_v, tokb_v, os_v, o1_v, o2_v, acc1_v, acc2_v,
               bl_v, x1_v, t_v, out_v, zs, sems):
        srcs = [wq_hbm, wk_hbm, wv_hbm]
        rings = [rq_v, rk_v, rv_v]
        muls = [scale, None, None]
        S_X0, S_X1, S_MEM, S_B, S_OUT, S_ST, S_ST2 = 0, 1, 2, 3, 7, 8, 11

        cp_x0 = pltpu.make_async_copy(x_hbm.at[0, pl.ds(0, L0)], x_v.at[pl.ds(0, L0)], sems.at[S_X0])
        cp_m = pltpu.make_async_copy(mem0_hbm.at[0], mem_v, sems.at[S_MEM])

        def unit_cp(g, w):
            return pltpu.make_async_copy(srcs[w].at[:, pl.ds(pl.multiple_of(g * HG, HG), HG), :], stage.at[w],
                                         sems.at[S_ST + w])

        R2 = stage2.shape[1]

        NCV = R2 // 16
        NCH = H * E // 16

        def wo_cp(i):
            sl = jax.lax.rem(i, 2)
            r0 = pl.multiple_of(jnp.minimum(i * R2, H * E - R2), 16)
            return pltpu.make_async_copy(wo_hbm.at[pl.ds(r0, R2)], stage2.at[sl], sems.at[S_ST2 + sl])

        def chunks(src_ref, dst_ref, nrows, n, sem, row0=0):
            r = nrows // n
            return [pltpu.make_async_copy(src_ref.at[pl.ds(row0 + c * r, r)], dst_ref.at[pl.ds(row0 + c * r, r)], sem)
                    for c in range(n)]

        x1_cps = chunks(x_hbm.at[0], x_v, S - L0, 3, sems.at[S_X1], L0)
        w1_cps = chunks(w1_hbm, w1_v, D, 2, sems.at[S_B])
        w2_cps = chunks(w2_hbm, w2_v, D, 2, sems.at[S_B + 1])
        w3_cps = chunks(w3_hbm, w3_v, D, 4, sems.at[S_B + 2])
        w4_cps = chunks(w4_hbm, w4_v, FF, 2, sems.at[S_B + 3])
        extra = {2 + j: cp for j, cp in enumerate(x1_cps + w1_cps + w2_cps + w3_cps[:2])}
        late = w3_cps[2:] + w4_cps

        zs[0] = 0
        zs[1] = 0
        cp_x0.start()
        cp_m.start()
        for w in range(3):
            unit_cp(0, w).start()
        wo_cp(0).start()
        stage2[1] = jnp.zeros(stage2.shape[1:], BF16)
        h1_v[pl.ds(0, PH), :] = jnp.zeros((PH, D), F32)
        h1_v[pl.ds(PH + S, PH), :] = jnp.zeros((PH, D), F32)
        cp_x0.wait()

        def ln_body(i, c):
            r0 = pl.multiple_of(i * 32, 32)
            xn0_v[pl.ds(pl.multiple_of(i * 16, 16), 16), :] = _u(_ln(x_v[pl.ds(r0, 32), :].astype(F32)).astype(BF16))
            return c
        jax.lax.fori_loop(0, L0 // 32, ln_body, 0)

        def relayout(g, w, t):
            v = stage[w, pl.ds(pl.multiple_of(t * 16, 16), 16)]
            wall_v[w + zs[0], pl.ds(pl.multiple_of(g * HG, HG), HG), pl.ds(pl.multiple_of(t * 8, 8), 8), :] = (
                _u(jnp.swapaxes(v, 0, 1)))

        NRL = D // 16
        unit_cp(0, 0).wait()

        def rl0(t, c):
            for u in range(4):
                relayout(0, 0, t * 4 + u)
            return c
        jax.lax.fori_loop(0, NRL // 4, rl0, 0)
        unit_cp(1, 0).start()

        NU = 3 * NG

        def pro_body(u, c):
            g = u // 3
            w = jax.lax.rem(u, 3)
            un = jnp.where(u + 1 < NU, u + 1, NU - 3)
            gn = un // 3
            wn = jax.lax.rem(un, 3)
            sl2 = jax.lax.rem(u + 1, 2)
            c0 = jnp.clip((u - 1) * NCV, 0, NCH - NCV)
            mul = jnp.where(w == 0, scale, 1.0).astype(F32)
            wvec = jnp.full((PM // 2, E), w, jnp.int32)
            msk = [wvec == w_ for w_ in range(3)]

            for w_ in range(3):
                @pl.when(jnp.logical_and(wn == w_, u + 1 < NU))
                def _(w_=w_):
                    unit_cp(gn, w_).wait()

            @pl.when(u >= 1)
            def _():
                wo_cp(u - 1).wait()
            ND = HG * (L0 // PM) * KS - PSKIP
            KW = D // KS
            n = 0
            for j in range(HG):
                h = g * HG + j
                for mb in range(L0 // PM):
                    y = None
                    for ks in range(KS):
                        yk = _dot(_b(xn0_v[pl.ds(mb * PM // 2, PM // 2), ks * KW:(ks + 1) * KW]),
                                  _b(wall_v[w + zs[1], h, pl.ds(ks * KW // 2, KW // 2), :]))
                        y = yk if y is None else y + yk
                        if ks == KS - 1:
                            yb = _u((y * mul).astype(BF16))
                            for w_ in range(3):
                                pltpu.store(rings[w_].at[h, pl.ds((ROFF + mb * PM) // 2, PM // 2), :], yb,
                                            mask=msk[w_])
                        for t in range(min(n, ND) * NRL // ND, min(n + 1, ND) * NRL // ND):
                            relayout(gn, wn, t)
                        for t in range(min(n, ND) * NCV // ND, min(n + 1, ND) * NCV // ND):
                            ch = c0 + t
                            hh = ch // (E // 16)
                            tr = pl.multiple_of(jax.lax.rem(ch, E // 16) * 8, 8)
                            cvt = _u(stage2[sl2, pl.ds(t * 16, 16), :])
                            for nn in range(NT):
                                wall_v[3 + zs[0], hh, pl.ds(nn * (E // 2) + tr, 8), :] = (
                                    cvt[:, nn * 128:(nn + 1) * 128])
                        n += 1

            @pl.when(u + 1 < NWO)
            def _():
                wo_cp(u + 1).start()
            for w_ in range(3):
                @pl.when(jnp.logical_and(wn == w_, u + 4 < NU))
                def _(w_=w_):
                    unit_cp(gn + 1, w_).start()
            for it_, cp_ in extra.items():
                @pl.when(u == it_)
                def _(cp_=cp_):
                    cp_.start()
            return c
        NWO = -(-NCH // NCV)
        assert NWO == NU - 1
        jax.lax.fori_loop(0, NU, pro_body, 0)
        for cp in late:
            cp.start()
        cp_m.wait()
        for cp in x1_cps:
            cp.wait()

        P2 = 2 * SEG + 2 * M
        row = jax.lax.broadcasted_iota(jnp.int32, (P2, P2), 0)
        col = jax.lax.broadcasted_iota(jnp.int32, (P2, P2), 1)

        def head_of(z):
            return jnp.where(z < 2 * SEG, z // SEG, (z - 2 * SEG) // M)
        causal = jax.lax.rem(col, SEG) <= jax.lax.rem(row, SEG)
        allowed = (head_of(row) == head_of(col)) & ((row >= 2 * SEG) | (col >= 2 * SEG) | causal)

        def ln_tokens(t0):
            return _ln(x_v[pl.ds(pl.multiple_of(t0, 8), TP), :].astype(F32))

        def set_lhs(lhs_v, t0, mem):
            lhs_v[...] = _u(jnp.concatenate([ln_tokens(t0), mem], axis=0).astype(BF16))

        def prep_lhs(lhs_v, slot, t0):
            t = ln_tokens(t0)
            lhs_v[pl.ds(0, 8), :] = _u(t[0:16].astype(BF16))
            tokb_v[slot] = t[16:24]

        def finish_lhs(lhs_v, slot, mem):
            lhs_v[pl.ds(8, 8), :] = _u(jnp.concatenate([tokb_v[slot], mem], axis=0).astype(BF16))

        def b_ops(j1, j2):
            r1 = pl.multiple_of(j1 * RB, RB)
            r2 = pl.multiple_of(j2 * RB, RB)
            part = {}

            def half_dot(lhs_ref, w_ref, n, hf):
                return _dot(_b(lhs_ref[:, hf * KH:(hf + 1) * KH]),
                            w_ref[hf * KH:(hf + 1) * KH, n * 128:(n + 1) * 128])

            def ln1(c):
                a = _ln(_ln(h_v[pl.ds(r1 + 16 * c, 8), :]))
                b = _ln(_ln(h_v[pl.ds(r1 + 16 * c + 8, 8), :]))
                bl_v[0, pl.ds(8 * c, 8), :] = _u(jnp.concatenate([a, b], axis=0).astype(BF16))

            def w1(n, hf):
                y = half_dot(bl_v.at[0], w1_v, n, hf)
                if hf == 0:
                    part['w1'] = y
                else:
                    h1_v[pl.ds(r1 + PH, RB), n * 128:(n + 1) * 128] = _gelu(part.pop('w1') + y)

            def mix(g):
                off = (-1, 1, -2, 2)[g]
                lo = 0 if off < 0 else PH
                win = h1_v[pl.ds(r2 + lo, RB + PH), g * C4:(g + 1) * C4]
                s0 = PH + off - lo
                bl_v[1, :, g * C4:(g + 1) * C4] = _u(win[s0:s0 + RB].astype(BF16))

            def w2(n, hf):
                y = None
                for g in (hf, hf + 2):
                    yg = _dot(_b(bl_v[1, :, g * C4:(g + 1) * C4]), w2_v[g * C4:(g + 1) * C4, n * 128:(n + 1) * 128])
                    y = yg if y is None else y + yg
                if hf == 0:
                    x1_v[:, n * 128:(n + 1) * 128] = y
                else:
                    x1_v[:, n * 128:(n + 1) * 128] += y

            def ln2(c):
                res = []
                for hf in range(2):
                    rows = pl.ds(16 * c + 8 * hf, 8)
                    hb = h_v[pl.ds(r2 + 16 * c + 8 * hf, 8), :]
                    x1 = _ln(hb) + x1_v[rows, :]
                    x1_v[rows, :] = hb + x1
                    res.append(_ln(x1))
                bl_v[2, pl.ds(8 * c, 8), :] = _u(jnp.concatenate(res, axis=0).astype(BF16))

            def w3(n, hf):
                y = half_dot(bl_v.at[2], w3_v, n, hf)
                if hf == 0:
                    part['w3'] = y
                else:
                    t_v[:, n * 128:(n + 1) * 128] = _u(_gelu(part.pop('w3') + y).astype(BF16))

            def w4(gi, n, pc):
                k0 = gi * D + pc * KH
                y = _dot(_b(t_v[:, k0:k0 + KH]), w4_v[k0:k0 + KH, n * 128:(n + 1) * 128])
                if gi < 3 and pc == 0:
                    part['w4'] = y
                    return
                if gi < 3:
                    y = part.pop('w4') + y
                y = x1_v[:, n * 128:(n + 1) * 128] + y
                if gi < 3:
                    x1_v[:, n * 128:(n + 1) * 128] = y
                else:
                    out_v[pl.ds(r2, RB), n * 128:(n + 1) * 128] = y.astype(BF16)

            return dict(ln1=ln1, w1=w1, mix=mix, w2=w2, ln2=ln2, w3=w3, w4=w4)

        def phase(p, k, bops):
            lhs_v = lhs2_v if p == 2 else lhs1_v
            o_v = o1_v if p == 1 else o2_v
            acc_v = acc1_v if p == 1 else acc2_v
            if p == 0:
                odd = jax.lax.rem(k, 2)
                wbase = pl.multiple_of((k // 2) * TP, 8)
                rbase = pl.multiple_of(k * (SEG // 2) + ROFF // 2, SEG // 2)
                keep_new = jax.lax.broadcasted_iota(jnp.int32, (8, E), 0) // 4 == odd
            else:
                wbase = pl.multiple_of(jax.lax.rem(k * TP, R // 2), 8)
                rbase = pl.multiple_of(jax.lax.rem(k * SEG + (p - 1) * (SEG // 2) + ROFF // 2, R // 2), SEG // 2)
            memf, pb, rinv, toks = {}, {}, {}, {}

            def proj(w, h):
                y = _dot(_b(lhs_v[...]), _b(wall_v[w, h]))
                if muls[w] is not None:
                    y = y * muls[w]
                view = rings[w].at[h, pl.ds(wbase, TP)]
                if p == 1:
                    view[pl.ds(0, 8), :] = _u(y[0:16].astype(BF16))
                    view[pl.ds(8, 4), :] = _u(y[16:32].astype(BF16))[0:4]
                elif p == 2:
                    view[pl.ds(12, 4), :] = _u(jnp.concatenate([y[0:8], y[0:8]], axis=0).astype(BF16))[4:8]
                    view[pl.ds(16, 8), :] = _u(y[8:24].astype(BF16))
                else:
                    is_odd = odd == 1
                    fullv = jnp.where(is_odd, _u(y[8:24].astype(BF16)), _u(y[0:16].astype(BF16)))
                    halfv = jnp.where(is_odd, _u(jnp.concatenate([y[0:8], y[0:8]], axis=0).astype(BF16)),
                                      _u(y[16:32].astype(BF16)))
                    view[pl.ds(pl.multiple_of(odd * 16, 8), 8), :] = fullv
                    view[pl.ds(8, 8), :] = jnp.where(keep_new, halfv, view[pl.ds(8, 8), :])
                memf[(w, h)] = y[TP:TP + M]

            def load_tok(w, j):
                toks[(w, j)] = [_b(rings[w][2 * j + a, pl.ds(rbase, SEG // 2), :]) for a in range(2)]

            def full(w, j):
                mem16 = jnp.concatenate([memf.pop((w, 2 * j)), memf.pop((w, 2 * j + 1))], axis=0).astype(BF16)
                return jnp.concatenate(toks.pop((w, j)) + [mem16], axis=0)

            def qk(j):
                load_tok(1, j)
                sc = jax.lax.dot_general(full(0, j), full(1, j), (((1,), (1,)), ((), ())),
                                         preferred_element_type=F32)
                sc = jnp.where(allowed, sc, -1e30)
                pe = jnp.exp(sc - jnp.max(sc, axis=-1, keepdims=True))
                rinv[j] = pl.reciprocal(jnp.sum(pe, axis=-1, keepdims=True), approx=False)
                pb[j] = pe.astype(BF16)

            def pv(j):
                load_tok(2, j)
                o2 = _dot(pb.pop(j), full(2, j)) * rinv.pop(j)
                for a in range(2):
                    ot = o2[a * SEG:(a + 1) * SEG]
                    om = o2[2 * SEG + a * M:2 * SEG + (a + 1) * M]
                    cs = slice((2 * j + a) * E, (2 * j + a + 1) * E)
                    if p == 0:
                        o_v[:, cs] = _u(jnp.concatenate([ot, om, jnp.zeros((8, E), F32)], axis=0).astype(BF16))
                    elif p == 1:
                        o_v[:, cs] = _u(jnp.concatenate([ot[0:24], om], axis=0).astype(BF16))
                        os_v[:, cs] = ot[24:32]
                    else:
                        o_v[:, cs] = _u(jnp.concatenate([ot, om, os_v[:, cs]], axis=0).astype(BF16))

            def wo_group(g):
                ogs = [_b(o_v[:, (g * G + j) * E:(g * G + j + 1) * E]) for j in range(G)]
                for n in range(NT):
                    y = None
                    for j in range(G):
                        yj = _dot(ogs[j], _b(wall_v[3, g * G + j, pl.ds(n * (E // 2), E // 2), :]))
                        y = yj if y is None else y + yj
                    if g == 0:
                        acc_v[:, n * 128:(n + 1) * 128] = y
                    else:
                        acc_v[:, n * 128:(n + 1) * 128] += y

            def fin():
                if p == 0:
                    r0 = pl.multiple_of(k * SEG, SEG)
                    h_v[pl.ds(r0, SEG), :] = x_v[pl.ds(r0, SEG), :].astype(F32) + acc_v[pl.ds(0, SEG), :]
                    set_lhs(lhs1_v, L0 + (k + 1) * TP, acc_v[pl.ds(32, 8), :])
                    return
                r0 = pl.multiple_of(k * RB, RB)
                if p == 1:
                    h_v[pl.ds(r0, 24), :] = x_v[pl.ds(r0, 32), :].astype(F32)[0:24] + acc_v[pl.ds(0, 24), :]
                    finish_lhs(lhs2_v, 0, acc_v[pl.ds(24, 8), :])
                else:
                    xa = x_v[pl.ds(r0 + 16, 16), :].astype(F32)[8:16]
                    h_v[pl.ds(r0 + 24, 8), :] = xa + acc_v[pl.ds(40, 8), :]
                    h_v[pl.ds(r0 + 32, 32), :] = x_v[pl.ds(r0 + 32, 32), :].astype(F32) + acc_v[pl.ds(0, 32), :]
                    finish_lhs(lhs1_v, 1, acc_v[pl.ds(32, 8), :])

            def emit_b(it, sl):
                if bops is None:
                    return
                for op in sched.get((p, it, sl), []):
                    if op[0] == 'prep':
                        tnext = L0 + k * (2 * TP) + TP * p
                        if p == 1:
                            prep_lhs(lhs2_v, 0, tnext)
                        else:
                            prep_lhs(lhs1_v, 1, jnp.minimum(tnext, S - TP))
                    else:
                        bops[op[0]](*op[1:])

            NIT = H + LP
            for it in range(NIT):
                jq = (it - LQ) // 2 if (it - LQ) % 2 == 0 and 0 <= it - LQ < H else None
                jp = (it - LP) // 2 if (it - LP) % 2 == 0 and 0 <= it - LP < H else None
                if jq is not None:
                    load_tok(0, jq)
                if it < H:
                    proj(0, it)
                    emit_b(it, 0)
                if jq is not None:
                    qk(jq)
                if it >= H:
                    emit_b(it, 0)
                if it < H:
                    proj(1, it)
                    emit_b(it, 1)
                if jp is not None:
                    pv(jp)
                if it >= H:
                    emit_b(it, 1)
                if it < H:
                    proj(2, it)
                hd = it - LP
                if 0 <= hd < H and hd % G == G - 1:
                    wo_group(hd // G)
                if it == NIT - 1:
                    fin()
                emit_b(it, 2)

        def out_cp(j):
            r = pl.multiple_of(j * RB, RB)
            return pltpu.make_async_copy(out_v.at[pl.ds(r, RB)], out_hbm.at[0, pl.ds(r, RB)], sems.at[S_OUT])

        def run_ops(bops, names):
            for op in names:
                bops[op[0]](*op[1:])

        def a_body(s, c):
            phase(0, s, None)
            return c

        def sup_body(k, c):
            bops = b_ops(k - 1, k - 2)
            phase(1, k, bops)
            phase(2, k, bops)
            out_cp(k - 2).start()
            return c

        st1 = [('ln1', c) for c in range(4)] + [('w1', n, hf) for n in range(NT) for hf in range(2)]
        st2 = ([('mix', g) for g in (0, 2, 1, 3)] + [('w2', n, hf) for hf in range(2) for n in range(NT)]
               + [('ln2', c) for c in range(4)] + [('w3', n, hf) for n in range(NF) for hf in range(2)]
               + [('w4', gi, n, pc) for gi in range(4) for n in range(NT) for pc in range(2 if gi < 3 else 1)])

        set_lhs(lhs1_v, L0, mem_v[...].astype(F32))
        jax.lax.fori_loop(0, 4, a_body, 0)
        for cp in w1_cps:
            cp.wait()
        run_ops(b_ops(0, 0), st1)
        for cp in w2_cps + w3_cps + w4_cps:
            cp.wait()
        jax.lax.fori_loop(2, NSUP, sup_body, 0)

        run_ops(b_ops(NSUP - 1, NSUP - 1), st1)

        def epi_body(j, c):
            run_ops(b_ops(j, j), st2)
            out_cp(j).start()
            return c
        jax.lax.fori_loop(NSUP - 2, NSUP, epi_body, 0)
        for j in range(NSUP):
            out_cp(j).wait()

    scratch = [
        pltpu.VMEM((S, D), BF16),
        pltpu.VMEM((L0 // 2, D), U32),
        pltpu.VMEM((S, D), F32),
        pltpu.VMEM((PH + S + PH, D), F32),
        pltpu.VMEM((4, H, D // 2, E), U32),
        pltpu.VMEM((D, D), BF16), pltpu.VMEM((D, D), BF16), pltpu.VMEM((D, FF), BF16), pltpu.VMEM((FF, D), BF16),
        pltpu.VMEM((3, D, HG, E), BF16),
        pltpu.VMEM((2, 384, D), BF16),
        pltpu.VMEM((M, D), BF16),
        pltpu.VMEM((H, R // 2, E), U32), pltpu.VMEM((H, R // 2, E), U32), pltpu.VMEM((H, R // 2, E), U32),
        pltpu.VMEM((16, D), U32),
        pltpu.VMEM((16, D), U32),
        pltpu.VMEM((2, 8, D), F32),
        pltpu.VMEM((8, H * E), F32),
        pltpu.VMEM((16, H * E), U32),
        pltpu.VMEM((24, H * E), U32),
        pltpu.VMEM((32, D), F32),
        pltpu.VMEM((48, D), F32),
        pltpu.VMEM((3, RB // 2, D), U32),
        pltpu.VMEM((RB, D), F32),
        pltpu.VMEM((RB // 2, FF), U32),
        pltpu.VMEM((S, D), BF16),
        pltpu.SMEM((2,), jnp.int32),
        pltpu.SemaphoreType.DMA((13,)),
    ]
    return kernel, scratch


@functools.partial(jax.jit, static_argnames=("A_seg_len",))
def pallas_sequential_preLN__memory_aug_recurrent_mem_tr__mixer_s_mlp__prompt_kernel(
        A_x, A_mem0, A_Wq, A_Wk, A_Wv, A_Wo, A_seg_len, B_x, B_w1, B_w2, B_w3, B_w4):
    del B_x
    B, S, D = A_x.shape
    _, H, E = A_Wq.shape
    assert B == 1
    kernel, scratch = _make_kernel(S, D, H, E, A_mem0.shape[1], int(A_seg_len), B_w3.shape[1])
    any_spec = pl.BlockSpec(memory_space=pl.ANY)
    return pl.pallas_call(
        kernel,
        out_shape=jax.ShapeDtypeStruct((B, S, D), BF16),
        in_specs=[any_spec] * 10,
        out_specs=any_spec,
        scratch_shapes=scratch,
        compiler_params=pltpu.CompilerParams(vmem_limit_bytes=120 * 1024 * 1024, disable_bounds_checks=True),
    )(A_x, A_mem0, A_Wq, A_Wk, A_Wv, A_Wo.reshape(H * E, D), B_w1, B_w2, B_w3, B_w4)
```

```python
import functools

import jax
import jax.numpy as jnp
from jax.experimental import pallas as pl
from jax.experimental.pallas import tpu as pltpu

F32 = jnp.float32
BF16 = jnp.bfloat16
U32 = jnp.uint32
EPS = 1e-5


def _ln(x):
    m = jnp.mean(x, axis=-1, keepdims=True)
    xc = x - m
    v = jnp.mean(xc * xc, axis=-1, keepdims=True)
    return xc * jax.lax.rsqrt(v + EPS)


def _gelu(x):
    c = 0.7978845608028654
    return 0.5 * x * (1.0 + jnp.tanh(c * (x + 0.044715 * (x * x * x))))


def _dot(a, b):
    return jnp.dot(a, b, preferred_element_type=F32)


def _b(x):
    return pltpu.bitcast(x, BF16)


def _u(x):
    return pltpu.bitcast(x, U32)


def _mixer_schedule(H):
    s = {}

    def add(p, it, sl, op):
        s.setdefault((p, it, sl), []).append(op)

    def spread(ops, positions):
        assert len(ops) == len(positions), (len(ops), len(positions))
        for op, (p, it, sl) in zip(ops, positions):
            add(p, it, sl, op)

    def two(p, lo, hi):
        return [(p, it, sl) for it in range(lo, hi) for sl in (0, 1)]

    def tail(p):
        return [(p, H, 0)] * 3 + [(p, H + 1, 0)] * 2 + [(p, H + 2, 1)] * 4 + [(p, H + 3, 2)] * 4

    add(1, 0, 0, ('mix', 0))
    add(1, 0, 0, ('mix', 2))
    for c in range(4):
        add(1, c // 2, 2, ('ln1', c))
    spread([('w2', n, 0) for n in range(8)], two(1, 1, 5))
    spread([('w1', n, hf) for n in range(8) for hf in range(2)], two(1, 5, 13))
    add(1, 10, 2, ('mix', 1))
    add(1, 15, 2, ('mix', 3))
    spread([('w2', n, 1) for n in range(8)], two(1, 16, 20))
    for c in range(4):
        add(1, 20 + c, 2, ('ln2', c))
    for p in (1, 2):
        add(p, 8, 2, ('prep',))
    w3 = [('w3', n, hf) for n in range(28) for hf in range(2)]
    pos3 = two(1, 24, H) + tail(1)
    pos3 = pos3 + two(2, 0, H)[:len(w3) - len(pos3)]
    spread(w3, pos3)
    first = max(x[1] for x in pos3 if x[0] == 2) + 2
    w4 = [('w4', gi, n, pc) for gi in range(4) for n in range(8) for pc in range(2 if gi < 3 else 1)]
    its = list(range(first, H))
    extra = len(w4) - len(tail(2)) - 2 * len(its)
    pos4 = []
    for i, it in enumerate(its):
        pos4 += [(2, it, 0), (2, it, 1)] + ([(2, it, 2)] if i >= len(its) - extra else [])
    spread(w4, pos4 + tail(2))

    slot_order = {0: 0, 1: 1, 2: 2}
    seq = [op for key in sorted(s, key=lambda k: (k[0], k[1], slot_order[k[2]])) for op in s[key]]
    pos = {op: i for i, op in enumerate(seq)}
    last = lambda name: max(i for op, i in pos.items() if op[0] == name)
    first_ = lambda name: min(i for op, i in pos.items() if op[0] == name)
    assert last('ln1') < first_('w1') and last('w2') < first_('ln2') and last('ln2') < first_('w3')
    assert pos[('w1', 3, 1)] < pos[('mix', 1)] and pos[('w1', 7, 1)] < pos[('mix', 3)]
    assert max(pos[('mix', 0)], pos[('mix', 2)]) < min(pos[('w2', n, 0)] for n in range(8))
    assert max(pos[('mix', 1)], pos[('mix', 3)]) < min(pos[('w2', n, 1)] for n in range(8))
    assert all(pos[('w2', n, 0)] < pos[('w2', n, 1)] for n in range(8))
    for gi in range(4):
        assert pos[('w3', min(8 * gi + 7, 27), 1)] < min(i for op, i in pos.items() if op[0] == 'w4' and op[1] == gi)
    return s


def _make_kernel(S, D, H, E, M, SEG, FF):
    assert (SEG, M, E, H, D, FF) == (32, 8, 128, 32, 1024, 3584) and S == 2048
    NSEG = S // SEG
    NSUP = NSEG // 2
    RB = 2 * SEG
    TP = 24
    L0 = S - NSEG * TP
    R = 576
    ROFF = 64
    assert L0 == 512 and (L0 + ROFF) % R == 0 and R % (2 * TP) == 0 and R % SEG == 0
    scale = float(E) ** -0.5
    NT = D // 128
    NF = FF // 128
    PH = 8
    C4 = D // 4
    KH = D // 2
    HG = 8
    NG = H // HG
    PM = 128
    KS = 4
    PSKIP = 6
    G = 2
    LQ, LP = 2, 4
    sched = _mixer_schedule(H)

    def kernel(x_hbm, mem0_hbm, wq_hbm, wk_hbm, wv_hbm, wo_hbm, w1_hbm, w2_hbm, w3_hbm, w4_hbm,
               out_hbm,
               x_v, xn0_v, h_v, h1_v, wall_v, w1_v, w2_v, w3_v, w4_v,
               stage, stage2, mem_v, rq_v, rk_v, rv_v, lhs1_v, lhs2_v, tokb_v, os_v, o1_v, o2_v, acc1_v, acc2_v,
               bl_v, x1_v, t_v, out_v, zs, sems):
        srcs = [wq_hbm, wk_hbm, wv_hbm]
        rings = [rq_v, rk_v, rv_v]
        muls = [scale, None, None]
        S_X0, S_X1, S_MEM, S_B, S_OUT, S_ST, S_ST2 = 0, 1, 2, 3, 7, 8, 11

        cp_x0 = pltpu.make_async_copy(x_hbm.at[0, pl.ds(0, L0)], x_v.at[pl.ds(0, L0)], sems.at[S_X0])
        cp_m = pltpu.make_async_copy(mem0_hbm.at[0], mem_v, sems.at[S_MEM])

        def unit_cp(g, w):
            return pltpu.make_async_copy(srcs[w].at[:, pl.ds(pl.multiple_of(g * HG, HG), HG), :], stage.at[w],
                                         sems.at[S_ST + w])

        R2 = stage2.shape[1]

        NCV = R2 // 16
        NCH = H * E // 16

        def wo_cp(i):
            sl = jax.lax.rem(i, 2)
            r0 = pl.multiple_of(jnp.minimum(i * R2, H * E - R2), 16)
            return pltpu.make_async_copy(wo_hbm.at[pl.ds(r0, R2)], stage2.at[sl], sems.at[S_ST2 + sl])

        def chunks(src_ref, dst_ref, nrows, n, sem, row0=0):
            r = nrows // n
            return [pltpu.make_async_copy(src_ref.at[pl.ds(row0 + c * r, r)], dst_ref.at[pl.ds(row0 + c * r, r)], sem)
                    for c in range(n)]

        x1_cps = chunks(x_hbm.at[0], x_v, S - L0, 3, sems.at[S_X1], L0)
        w1_cps = chunks(w1_hbm, w1_v, D, 2, sems.at[S_B])
        w2_cps = chunks(w2_hbm, w2_v, D, 2, sems.at[S_B + 1])
        w3_cps = chunks(w3_hbm, w3_v, D, 4, sems.at[S_B + 2])
        w4_cps = chunks(w4_hbm, w4_v, FF, 2, sems.at[S_B + 3])
        extra = {2 + j: cp for j, cp in enumerate(x1_cps + w1_cps + w2_cps + w3_cps[:2])}
        late = w3_cps[2:] + w4_cps

        zs[0] = 0
        zs[1] = 0
        cp_x0.start()
        cp_m.start()
        for w in range(3):
            unit_cp(0, w).start()
        wo_cp(0).start()
        stage2[1] = jnp.zeros(stage2.shape[1:], BF16)
        h1_v[pl.ds(0, PH), :] = jnp.zeros((PH, D), F32)
        h1_v[pl.ds(PH + S, PH), :] = jnp.zeros((PH, D), F32)
        cp_x0.wait()

        def ln_body(i, c):
            r0 = pl.multiple_of(i * 32, 32)
            xn0_v[pl.ds(pl.multiple_of(i * 16, 16), 16), :] = _u(_ln(x_v[pl.ds(r0, 32), :].astype(F32)).astype(BF16))
            return c
        jax.lax.fori_loop(0, L0 // 32, ln_body, 0)

        def relayout(g, w, t):
            v = stage[w, pl.ds(pl.multiple_of(t * 16, 16), 16)]
            wall_v[w + zs[0], pl.ds(pl.multiple_of(g * HG, HG), HG), pl.ds(pl.multiple_of(t * 8, 8), 8), :] = (
                _u(jnp.swapaxes(v, 0, 1)))

        NRL = D // 16
        unit_cp(0, 0).wait()

        def rl0(t, c):
            for u in range(4):
                relayout(0, 0, t * 4 + u)
            return c
        jax.lax.fori_loop(0, NRL // 4, rl0, 0)
        unit_cp(1, 0).start()

        NU = 3 * NG

        def pro_body(u, c):
            g = u // 3
            w = jax.lax.rem(u, 3)
            un = jnp.where(u + 1 < NU, u + 1, NU - 3)
            gn = un // 3
            wn = jax.lax.rem(un, 3)
            sl2 = jax.lax.rem(u + 1, 2)
            c0 = jnp.clip((u - 1) * NCV, 0, NCH - NCV)
            mul = jnp.where(w == 0, scale, 1.0).astype(F32)
            wvec = jnp.full((PM // 2, E), w, jnp.int32)
            msk = [wvec == w_ for w_ in range(3)]

            for w_ in range(3):
                @pl.when(jnp.logical_and(wn == w_, u + 1 < NU))
                def _(w_=w_):
                    unit_cp(gn, w_).wait()

            @pl.when(u >= 1)
            def _():
                wo_cp(u - 1).wait()
            ND = HG * (L0 // PM) * KS - PSKIP
            KW = D // KS
            n = 0
            for j in range(HG):
                h = g * HG + j
                for mb in range(L0 // PM):
                    y = None
                    for ks in range(KS):
                        yk = _dot(_b(xn0_v[pl.ds(mb * PM // 2, PM // 2), ks * KW:(ks + 1) * KW]),
                                  _b(wall_v[w + zs[1], h, pl.ds(ks * KW // 2, KW // 2), :]))
                        y = yk if y is None else y + yk
                        if ks == KS - 1:
                            yb = _u((y * mul).astype(BF16))
                            for w_ in range(3):
                                pltpu.store(rings[w_].at[h, pl.ds((ROFF + mb * PM) // 2, PM // 2), :], yb,
                                            mask=msk[w_])
                        for t in range(min(n, ND) * NRL // ND, min(n + 1, ND) * NRL // ND):
                            relayout(gn, wn, t)
                        for t in range(min(n, ND) * NCV // ND, min(n + 1, ND) * NCV // ND):
                            ch = c0 + t
                            hh = ch // (E // 16)
                            tr = pl.multiple_of(jax.lax.rem(ch, E // 16) * 8, 8)
                            cvt = _u(stage2[sl2, pl.ds(t * 16, 16), :])
                            for nn in range(NT):
                                wall_v[3 + zs[0], hh, pl.ds(nn * (E // 2) + tr, 8), :] = (
                                    cvt[:, nn * 128:(nn + 1) * 128])
                        n += 1

            @pl.when(u + 1 < NWO)
            def _():
                wo_cp(u + 1).start()
            for w_ in range(3):
                @pl.when(jnp.logical_and(wn == w_, u + 4 < NU))
                def _(w_=w_):
                    unit_cp(gn + 1, w_).start()
            for it_, cp_ in extra.items():
                @pl.when(u == it_)
                def _(cp_=cp_):
                    cp_.start()
            return c
        NWO = -(-NCH // NCV)
        assert NWO == NU - 1
        jax.lax.fori_loop(0, NU, pro_body, 0)
        for cp in late:
            cp.start()
        cp_m.wait()
        for cp in x1_cps:
            cp.wait()

        P2 = 2 * SEG + 2 * M
        row = jax.lax.broadcasted_iota(jnp.int32, (P2, P2), 0)
        col = jax.lax.broadcasted_iota(jnp.int32, (P2, P2), 1)

        def head_of(z):
            return jnp.where(z < 2 * SEG, z // SEG, (z - 2 * SEG) // M)
        causal = jax.lax.rem(col, SEG) <= jax.lax.rem(row, SEG)
        same_head = head_of(row) == head_of(col)
        allowed = same_head & ((row >= 2 * SEG) | (col >= 2 * SEG) | causal)
        fill = jnp.where(same_head, -1e9, -1e30).astype(F32)

        def ln_tokens(t0):
            return _ln(x_v[pl.ds(pl.multiple_of(t0, 8), TP), :].astype(F32))

        def set_lhs(lhs_v, t0, mem):
            lhs_v[...] = _u(jnp.concatenate([ln_tokens(t0), mem], axis=0).astype(BF16))

        def prep_lhs(lhs_v, slot, t0):
            t = ln_tokens(t0)
            lhs_v[pl.ds(0, 8), :] = _u(t[0:16].astype(BF16))
            tokb_v[slot] = t[16:24]

        def finish_lhs(lhs_v, slot, mem):
            lhs_v[pl.ds(8, 8), :] = _u(jnp.concatenate([tokb_v[slot], mem], axis=0).astype(BF16))

        def b_ops(j1, j2):
            r1 = pl.multiple_of(j1 * RB, RB)
            r2 = pl.multiple_of(j2 * RB, RB)
            part = {}

            def half_dot(lhs_ref, w_ref, n, hf):
                return _dot(_b(lhs_ref[:, hf * KH:(hf + 1) * KH]),
                            w_ref[hf * KH:(hf + 1) * KH, n * 128:(n + 1) * 128])

            def ln1(c):
                a = _ln(_ln(h_v[pl.ds(r1 + 16 * c, 8), :]))
                b = _ln(_ln(h_v[pl.ds(r1 + 16 * c + 8, 8), :]))
                bl_v[0, pl.ds(8 * c, 8), :] = _u(jnp.concatenate([a, b], axis=0).astype(BF16))

            def w1(n, hf):
                y = half_dot(bl_v.at[0], w1_v, n, hf)
                if hf == 0:
                    part['w1'] = y
                else:
                    h1_v[pl.ds(r1 + PH, RB), n * 128:(n + 1) * 128] = _gelu(part.pop('w1') + y)

            def mix(g):
                off = (-1, 1, -2, 2)[g]
                lo = 0 if off < 0 else PH
                win = h1_v[pl.ds(r2 + lo, RB + PH), g * C4:(g + 1) * C4]
                s0 = PH + off - lo
                bl_v[1, :, g * C4:(g + 1) * C4] = _u(win[s0:s0 + RB].astype(BF16))

            def w2(n, hf):
                y = None
                for g in (hf, hf + 2):
                    yg = _dot(_b(bl_v[1, :, g * C4:(g + 1) * C4]), w2_v[g * C4:(g + 1) * C4, n * 128:(n + 1) * 128])
                    y = yg if y is None else y + yg
                if hf == 0:
                    x1_v[:, n * 128:(n + 1) * 128] = y
                else:
                    x1_v[:, n * 128:(n + 1) * 128] += y

            def ln2(c):
                res = []
                for hf in range(2):
                    rows = pl.ds(16 * c + 8 * hf, 8)
                    hb = h_v[pl.ds(r2 + 16 * c + 8 * hf, 8), :]
                    x1 = _ln(hb) + x1_v[rows, :]
                    x1_v[rows, :] = hb + x1
                    res.append(_ln(x1))
                bl_v[2, pl.ds(8 * c, 8), :] = _u(jnp.concatenate(res, axis=0).astype(BF16))

            def w3(n, hf):
                y = half_dot(bl_v.at[2], w3_v, n, hf)
                if hf == 0:
                    part['w3'] = y
                else:
                    t_v[:, n * 128:(n + 1) * 128] = _u(_gelu(part.pop('w3') + y).astype(BF16))

            def w4(gi, n, pc):
                k0 = gi * D + pc * KH
                y = _dot(_b(t_v[:, k0:k0 + KH]), w4_v[k0:k0 + KH, n * 128:(n + 1) * 128])
                if gi < 3 and pc == 0:
                    part['w4'] = y
                    return
                if gi < 3:
                    y = part.pop('w4') + y
                y = x1_v[:, n * 128:(n + 1) * 128] + y
                if gi < 3:
                    x1_v[:, n * 128:(n + 1) * 128] = y
                else:
                    out_v[pl.ds(r2, RB), n * 128:(n + 1) * 128] = y.astype(BF16)

            return dict(ln1=ln1, w1=w1, mix=mix, w2=w2, ln2=ln2, w3=w3, w4=w4)

        def phase(p, k, bops):
            lhs_v = lhs2_v if p == 2 else lhs1_v
            o_v = o1_v if p == 1 else o2_v
            acc_v = acc1_v if p == 1 else acc2_v
            if p == 0:
                odd = jax.lax.rem(k, 2)
                wbase = pl.multiple_of((k // 2) * TP, 8)
                rbase = pl.multiple_of(k * (SEG // 2) + ROFF // 2, SEG // 2)
                keep_new = jax.lax.broadcasted_iota(jnp.int32, (8, E), 0) // 4 == odd
            else:
                wbase = pl.multiple_of(jax.lax.rem(k * TP, R // 2), 8)
                rbase = pl.multiple_of(jax.lax.rem(k * SEG + (p - 1) * (SEG // 2) + ROFF // 2, R // 2), SEG // 2)
            memf, pb, rinv, toks = {}, {}, {}, {}

            def proj(w, h):
                y = _dot(_b(lhs_v[...]), _b(wall_v[w, h]))
                if muls[w] is not None:
                    y = y * muls[w]
                view = rings[w].at[h, pl.ds(wbase, TP)]
                if p == 1:
                    view[pl.ds(0, 8), :] = _u(y[0:16].astype(BF16))
                    view[pl.ds(8, 4), :] = _u(y[16:32].astype(BF16))[0:4]
                elif p == 2:
                    view[pl.ds(12, 4), :] = _u(jnp.concatenate([y[0:8], y[0:8]], axis=0).astype(BF16))[4:8]
                    view[pl.ds(16, 8), :] = _u(y[8:24].astype(BF16))
                else:
                    is_odd = odd == 1
                    fullv = jnp.where(is_odd, _u(y[8:24].astype(BF16)), _u(y[0:16].astype(BF16)))
                    halfv = jnp.where(is_odd, _u(jnp.concatenate([y[0:8], y[0:8]], axis=0).astype(BF16)),
                                      _u(y[16:32].astype(BF16)))
                    view[pl.ds(pl.multiple_of(odd * 16, 8), 8), :] = fullv
                    view[pl.ds(8, 8), :] = jnp.where(keep_new, halfv, view[pl.ds(8, 8), :])
                memf[(w, h)] = y[TP:TP + M]

            def load_tok(w, j):
                toks[(w, j)] = [_b(rings[w][2 * j + a, pl.ds(rbase, SEG // 2), :]) for a in range(2)]

            def full(w, j):
                mem16 = jnp.concatenate([memf.pop((w, 2 * j)), memf.pop((w, 2 * j + 1))], axis=0).astype(BF16)
                return jnp.concatenate(toks.pop((w, j)) + [mem16], axis=0)

            def qk(j):
                load_tok(1, j)
                sc = jax.lax.dot_general(full(0, j), full(1, j), (((1,), (1,)), ((), ())),
                                         preferred_element_type=F32)
                sc = jnp.where(allowed, sc, fill)
                pe = jnp.exp(sc - jnp.max(sc, axis=-1, keepdims=True))
                rinv[j] = pl.reciprocal(jnp.sum(pe, axis=-1, keepdims=True), approx=False)
                pb[j] = pe.astype(BF16)

            def pv(j):
                load_tok(2, j)
                o2 = _dot(pb.pop(j), full(2, j)) * rinv.pop(j)
                for a in range(2):
                    ot = o2[a * SEG:(a + 1) * SEG]
                    om = o2[2 * SEG + a * M:2 * SEG + (a + 1) * M]
                    cs = slice((2 * j + a) * E, (2 * j + a + 1) * E)
                    if p == 0:
                        o_v[:, cs] = _u(jnp.concatenate([ot, om, jnp.zeros((8, E), F32)], axis=0).astype(BF16))
                    elif p == 1:
                        o_v[:, cs] = _u(jnp.concatenate([ot[0:24], om], axis=0).astype(BF16))
                        os_v[:, cs] = ot[24:32]
                    else:
                        o_v[:, cs] = _u(jnp.concatenate([ot, om, os_v[:, cs]], axis=0).astype(BF16))

            def wo_group(g):
                ogs = [_b(o_v[:, (g * G + j) * E:(g * G + j + 1) * E]) for j in range(G)]
                for n in range(NT):
                    y = None
                    for j in range(G):
                        yj = _dot(ogs[j], _b(wall_v[3, g * G + j, pl.ds(n * (E // 2), E // 2), :]))
                        y = yj if y is None else y + yj
                    if g == 0:
                        acc_v[:, n * 128:(n + 1) * 128] = y
                    else:
                        acc_v[:, n * 128:(n + 1) * 128] += y

            def fin():
                if p == 0:
                    r0 = pl.multiple_of(k * SEG, SEG)
                    h_v[pl.ds(r0, SEG), :] = x_v[pl.ds(r0, SEG), :].astype(F32) + acc_v[pl.ds(0, SEG), :]
                    set_lhs(lhs1_v, L0 + (k + 1) * TP, acc_v[pl.ds(32, 8), :])
                    return
                r0 = pl.multiple_of(k * RB, RB)
                if p == 1:
                    h_v[pl.ds(r0, 24), :] = x_v[pl.ds(r0, 32), :].astype(F32)[0:24] + acc_v[pl.ds(0, 24), :]
                    finish_lhs(lhs2_v, 0, acc_v[pl.ds(24, 8), :])
                else:
                    xa = x_v[pl.ds(r0 + 16, 16), :].astype(F32)[8:16]
                    h_v[pl.ds(r0 + 24, 8), :] = xa + acc_v[pl.ds(40, 8), :]
                    h_v[pl.ds(r0 + 32, 32), :] = x_v[pl.ds(r0 + 32, 32), :].astype(F32) + acc_v[pl.ds(0, 32), :]
                    finish_lhs(lhs1_v, 1, acc_v[pl.ds(32, 8), :])

            def emit_b(it, sl):
                if bops is None:
                    return
                for op in sched.get((p, it, sl), []):
                    if op[0] == 'prep':
                        tnext = L0 + k * (2 * TP) + TP * p
                        if p == 1:
                            prep_lhs(lhs2_v, 0, tnext)
                        else:
                            prep_lhs(lhs1_v, 1, jnp.minimum(tnext, S - TP))
                    else:
                        bops[op[0]](*op[1:])

            NIT = H + LP
            for it in range(NIT):
                jq = (it - LQ) // 2 if (it - LQ) % 2 == 0 and 0 <= it - LQ < H else None
                jp = (it - LP) // 2 if (it - LP) % 2 == 0 and 0 <= it - LP < H else None
                if jq is not None:
                    load_tok(0, jq)
                if it < H:
                    proj(0, it)
                    emit_b(it, 0)
                if jq is not None:
                    qk(jq)
                if it >= H:
                    emit_b(it, 0)
                if it < H:
                    proj(1, it)
                    emit_b(it, 1)
                if jp is not None:
                    pv(jp)
                if it >= H:
                    emit_b(it, 1)
                if it < H:
                    proj(2, it)
                hd = it - LP
                if 0 <= hd < H and hd % G == G - 1:
                    wo_group(hd // G)
                if it == NIT - 1:
                    fin()
                emit_b(it, 2)

        def out_cp(j):
            r = pl.multiple_of(j * RB, RB)
            return pltpu.make_async_copy(out_v.at[pl.ds(r, RB)], out_hbm.at[0, pl.ds(r, RB)], sems.at[S_OUT])

        def run_ops(bops, names):
            for op in names:
                bops[op[0]](*op[1:])

        def a_body(s, c):
            phase(0, s, None)
            return c

        def sup_body(k, c):
            bops = b_ops(k - 1, k - 2)
            phase(1, k, bops)
            phase(2, k, bops)
            out_cp(k - 2).start()
            return c

        st1 = [('ln1', c) for c in range(4)] + [('w1', n, hf) for n in range(NT) for hf in range(2)]
        st2 = ([('mix', g) for g in (0, 2, 1, 3)] + [('w2', n, hf) for hf in range(2) for n in range(NT)]
               + [('ln2', c) for c in range(4)] + [('w3', n, hf) for n in range(NF) for hf in range(2)]
               + [('w4', gi, n, pc) for gi in range(4) for n in range(NT) for pc in range(2 if gi < 3 else 1)])

        set_lhs(lhs1_v, L0, mem_v[...].astype(F32))
        jax.lax.fori_loop(0, 4, a_body, 0)
        for cp in w1_cps:
            cp.wait()
        run_ops(b_ops(0, 0), st1)
        for cp in w2_cps + w3_cps + w4_cps:
            cp.wait()
        jax.lax.fori_loop(2, NSUP, sup_body, 0)

        run_ops(b_ops(NSUP - 1, NSUP - 1), st1)

        def epi_body(j, c):
            run_ops(b_ops(j, j), st2)
            out_cp(j).start()
            return c
        jax.lax.fori_loop(NSUP - 2, NSUP, epi_body, 0)
        for j in range(NSUP):
            out_cp(j).wait()

    scratch = [
        pltpu.VMEM((S, D), BF16),
        pltpu.VMEM((L0 // 2, D), U32),
        pltpu.VMEM((S, D), F32),
        pltpu.VMEM((PH + S + PH, D), F32),
        pltpu.VMEM((4, H, D // 2, E), U32),
        pltpu.VMEM((D, D), BF16), pltpu.VMEM((D, D), BF16), pltpu.VMEM((D, FF), BF16), pltpu.VMEM((FF, D), BF16),
        pltpu.VMEM((3, D, HG, E), BF16),
        pltpu.VMEM((2, 384, D), BF16),
        pltpu.VMEM((M, D), BF16),
        pltpu.VMEM((H, R // 2, E), U32), pltpu.VMEM((H, R // 2, E), U32), pltpu.VMEM((H, R // 2, E), U32),
        pltpu.VMEM((16, D), U32),
        pltpu.VMEM((16, D), U32),
        pltpu.VMEM((2, 8, D), F32),
        pltpu.VMEM((8, H * E), F32),
        pltpu.VMEM((16, H * E), U32),
        pltpu.VMEM((24, H * E), U32),
        pltpu.VMEM((32, D), F32),
        pltpu.VMEM((48, D), F32),
        pltpu.VMEM((3, RB // 2, D), U32),
        pltpu.VMEM((RB, D), F32),
        pltpu.VMEM((RB // 2, FF), U32),
        pltpu.VMEM((S, D), BF16),
        pltpu.SMEM((2,), jnp.int32),
        pltpu.SemaphoreType.DMA((13,)),
    ]
    return kernel, scratch


@functools.partial(jax.jit, static_argnames=("A_seg_len",))
def pallas_sequential_preLN__memory_aug_recurrent_mem_tr__mixer_s_mlp__prompt_kernel(
        A_x, A_mem0, A_Wq, A_Wk, A_Wv, A_Wo, A_seg_len, B_x, B_w1, B_w2, B_w3, B_w4):
    del B_x
    B, S, D = A_x.shape
    _, H, E = A_Wq.shape
    assert B == 1
    kernel, scratch = _make_kernel(S, D, H, E, A_mem0.shape[1], int(A_seg_len), B_w3.shape[1])
    any_spec = pl.BlockSpec(memory_space=pl.ANY)
    return pl.pallas_call(
        kernel,
        out_shape=jax.ShapeDtypeStruct((B, S, D), BF16),
        in_specs=[any_spec] * 10,
        out_specs=any_spec,
        scratch_shapes=scratch,
        compiler_params=pltpu.CompilerParams(vmem_limit_bytes=120 * 1024 * 1024, disable_bounds_checks=True),
    )(A_x, A_mem0, A_Wq, A_Wk, A_Wv, A_Wo.reshape(H * E, D), B_w1, B_w2, B_w3, B_w4)
```
